```python
import jax
import jax.numpy as jnp

def _softmax(x, axis=-1):
    return jax.nn.softmax(x, axis=axis)
def _gelu(x):
    return jax.nn.gelu(x, approximate=True)
def _silu(x):
    return jax.nn.silu(x)
def _sigmoid(x):
    return jax.nn.sigmoid(x)
def _layernorm(x, axis=-1, eps=1e-5):
    m = jnp.mean(x, axis=axis, keepdims=True)
    v = jnp.var(x, axis=axis, keepdims=True)
    return (x - m) / jnp.sqrt(v + eps)
def _scatter_add(tgt, idx, src, axis=0):
    return tgt.at[idx].add(src)
def _segment_sum(src, seg, n):
    return jax.ops.segment_sum(src, seg, n)
class _Rng:
    def __init__(self, key):
        self._k = key
    def _next(self):
        self._k, sub = jax.random.split(self._k)
        return sub
    def normal(self, shape):
        return jax.random.normal(self._next(), shape, dtype=jnp.bfloat16)
    def randint(self, lo, hi, shape):
        return jax.random.randint(self._next(), shape, lo, hi, dtype=jnp.int32)
    def uniform(self, shape, lo=0.0, hi=1.0):
        return jax.random.uniform(self._next(), shape, jnp.bfloat16, lo, hi)
    def permutation(self, n):
        return jax.random.permutation(self._next(), n)


kernel_name = 'recurrent_scan__gqa_block_cached__moe_arch_mod__prompt'

def setup_inputs():
    _rng = _Rng(jax.random.key(int.from_bytes(__import__("os").urandom(4), "little")))
    _w = (lambda a: (lambda t: t.astype(jnp.bfloat16) if jnp.issubdtype(t.dtype, jnp.floating) else t)(jnp.asarray(a)))
    def _A_setup():
        B, Sq, D = 1, 2048, 576
        Hq, Hkv, Sk, Dh = 32, 16, 2048, 128
        assert Hq % Hkv == 0, (Hq, Hkv)
        return {
            "x": _w((lambda *s: _rng.normal(s) * 0.05)(B, Sq, D)),
            "k_cache": _w((lambda *s: _rng.normal(s) * 0.05)(B, Hkv, Sk, Dh)),
            "v_cache": _w((lambda *s: _rng.normal(s) * 0.05)(B, Hkv, Sk, Dh)),
            "wq": _w((lambda *s: _rng.normal(s) * 0.05)(D, Hq * Dh) * (D ** -0.5)),
            "wo": _w((lambda *s: _rng.normal(s) * 0.05)(Hq * Dh, D) * ((Hq * Dh) ** -0.5)),
        }
    _A_in = _A_setup()

    def _B_setup():
        B, S, D, F, C = 1, 2048, 576, 4608, 8
        return {
            "x": _w((lambda *s: _rng.normal(s) * 0.05)(B, S, D)),
            "w_r": _w((lambda *s: _rng.normal(s) * 0.05)(D)),
            "w_gate": _w((lambda *s: _rng.normal(s) * 0.05)(D, F)),
            "w_up": _w((lambda *s: _rng.normal(s) * 0.05)(D, F)),
            "w_down": _w((lambda *s: _rng.normal(s) * 0.05)(F, D)),
        }
    _B_in = _B_setup()

    return {
        "A_x": _A_in["x"],
        "A_k_cache": _A_in["k_cache"],
        "A_v_cache": _A_in["v_cache"],
        "A_wq": _A_in["wq"],
        "A_wo": _A_in["wo"],
        "B_x": _B_in["x"],
        "B_w_r": _B_in["w_r"],
        "B_w_gate": _B_in["w_gate"],
        "B_w_up": _B_in["w_up"],
        "B_w_down": _B_in["w_down"],
    }

def reference(A_x, A_k_cache, A_v_cache, A_wq, A_wo, B_x, B_w_r, B_w_gate, B_w_up, B_w_down):
    def _A_ref(x, k_cache, v_cache, wq, wo):
        B, Sq, D = x.shape
        Hq, Dh = 32, 128
        Hkv = k_cache.shape[1]
        rep = Hq // Hkv
        q = (lambda x, *d: x.transpose(*d))((x @ wq).reshape(B, Sq, Hq, Dh), 0, 2, 1, 3)
        k = jnp.repeat(k_cache, rep, axis=1)
        v = jnp.repeat(v_cache, rep, axis=1)
        scores = jnp.einsum("bhqd,bhkd->bhqk", q, k) * (Dh ** -0.5)
        p = _softmax(scores, axis=-1)
        o = jnp.einsum("bhqk,bhkd->bhqd", p, v)
        return (lambda x, *d: x.transpose(*d))(o, 0, 2, 1, 3).reshape(B, Sq, Hq * Dh) @ wo

    def _B_ref(x, w_r, w_gate, w_up, w_down):
        B, S, D = x.shape
        C = 8
        r = x @ w_r
        idx = jnp.argsort(-r, axis=-1)[:, :C]
        idx_e = jnp.repeat(idx.reshape(B, C, 1), D, axis=2)
        x_sel = jnp.take_along_axis(x, idx_e, axis=1)
        g = _silu(x_sel @ w_gate)
        u = x_sel @ w_up
        y = (g * u) @ w_down
        r_sel = _sigmoid(jnp.take_along_axis(r, idx, axis=1))
        y = y * r_sel.reshape(B, C, 1)
        b_off = (jnp.arange(B) * S).reshape(B, 1)
        flat_idx = (idx + b_off).reshape(B * C)
        zero = (x * 0.0).reshape(B * S, D)
        upd = _scatter_add(zero, flat_idx, y.reshape(B * C, D), axis=0)
        return x + upd.reshape(B, S, D)

    x = A_x
    xn = _layernorm(x, axis=-1)
    s = _A_ref(xn, A_k_cache, A_v_cache, A_wq, A_wo)
    g = _silu(_B_ref(xn, B_w_r, B_w_gate, B_w_up, B_w_down))
    return x + s * g
```

```python
import functools
import math

import jax
import jax.numpy as jnp
from jax import lax
from jax.experimental import pallas as pl
from jax.experimental.pallas import tpu as pltpu

S = 2048
D = 576
HKV = 16
DH = 128
F = 4608
C = 8
EPS = 1e-5

NT = (((1,), (1,)), ((), ()))
BF = jnp.bfloat16
F32 = jnp.float32


def _rb(x):
    return x.astype(BF).astype(F32)


def _sigmoid(x):
    return 1.0 / (1.0 + jnp.exp(-x))


def make_kernel(TQ=512, TB=256, CK1=256, CK2=128, PVW=512, LNB=256, P1H=2):
    NQ = S // TQ
    LOG_NQ = int(math.log2(NQ))
    W = 2 * TQ
    U = HKV * NQ
    NB = S // TB
    QSCALE = (DH ** -0.5) * math.log2(math.e)

    def kernel(xt_hbm, k_hbm, v_hbm, wq_hbm, wot_hbm, wg_hbm, wu_hbm, wdt_hbm, wr_ref,
               o_hbm,
               xt_v, xnt_v, k_v, v_v, vt_v, wq_v, wot_v, qo_v,
               sa_v, sb_v, ma_v, mb_v, wg_v, wu_v, wdt_v, yb_v, idx_v, st_v, os_v,
               sem_x, sem_wq, sem_v, sem_k, sem_f, sem_o):

        def cp_x():
            return pltpu.make_async_copy(xt_hbm, xt_v, sem_x.at[0])

        def cp_wq(h):
            return pltpu.make_async_copy(
                wq_hbm.at[:, pl.ds(pl.multiple_of(h * 256, 256), 256)], wq_v.at[h], sem_wq.at[h])

        def cp_v(h):
            return pltpu.make_async_copy(v_hbm.at[h], v_v.at[h], sem_v.at[h])

        def cp_k(h):
            return pltpu.make_async_copy(k_hbm.at[h], k_v.at[h], sem_k.at[h])

        def cp_f(i):
            src, dst = ((wg_hbm, wg_v), (wu_hbm, wu_v), (wdt_hbm, wdt_v), (wot_hbm, wot_v))[i]
            return pltpu.make_async_copy(src, dst, sem_f.at[i])

        def cp_o(b, slot):
            return pltpu.make_async_copy(
                os_v.at[slot], o_hbm.at[:, pl.ds(pl.multiple_of(b * TB, TB), TB)], sem_o.at[slot])

        cp_x().start()
        cp_wq(0).start()
        with jax.named_scope('xwait'):
            cp_x().wait()
        for h in range(HKV):
            if h > 0:
                cp_wq(h).start()
            cp_v(h).start()
        for h in range(HKV):
            cp_k(h).start()
        for i in range(4):
            cp_f(i).start()

        def ln_body(b, c):
            cols = pl.ds(pl.multiple_of(b * LNB, LNB), LNB)
            x = xt_v[:, cols].astype(F32)
            mean = jnp.sum(x, axis=0, keepdims=True) * (1.0 / D)
            xc = x - mean
            var = jnp.sum(xc * xc, axis=0, keepdims=True) * (1.0 / D)
            den = _rb(jnp.sqrt(_rb(_rb(var) + EPS)))
            xn = _rb(x - _rb(mean)) * (1.0 / den)
            xnt_v[:, cols] = xn.astype(BF)
            return c
        with jax.named_scope('ln'):
            lax.fori_loop(0, S // LNB, ln_body, 0)

        def p1_body(t, c):
            for hh in range(P1H):
                h = t * P1H + hh
                cp_wq(h).wait()
                cp_v(h).wait()
            for hh in range(P1H):
                h = t * P1H + hh
                qt = jnp.dot(wq_v[h].T, xnt_v[...], preferred_element_type=F32) * QSCALE
                qt = qt.astype(BF)
                for i in range(NQ):
                    for a in range(2):
                        qo_v[h * NQ + i, :, a * TQ:(a + 1) * TQ] = qt[a * DH:(a + 1) * DH, i * TQ:(i + 1) * TQ]
                vt_v[h] = v_v[h].T
            return c
        with jax.named_scope('p1'):
            lax.fori_loop(0, HKV // P1H, p1_body, 0)

        def router_ffn():
            wr8 = jnp.broadcast_to(wr_ref[...], (C, D))
            r = _rb(jnp.dot(wr8, xnt_v[...], preferred_element_type=F32))
            tok = lax.broadcasted_iota(jnp.int32, (C, S), 1).astype(F32)
            row = lax.broadcasted_iota(jnp.int32, (C, 1), 0)
            idx = jnp.zeros((C, 1), F32)
            val = jnp.zeros((C, 1), F32)
            for c in range(C):
                mx = jnp.max(r, axis=1, keepdims=True)
                ix = jnp.min(jnp.where(r == mx, tok, float(S)), axis=1, keepdims=True)
                r = jnp.where(tok == ix, -jnp.inf, r)
                idx = jnp.where(row == c, ix, idx)
                val = jnp.where(row == c, mx, val)
            onehot = jnp.where(tok == idx, 1.0, 0.0).astype(BF)
            xs = lax.dot_general(onehot, xnt_v[...], NT, preferred_element_type=F32).astype(BF)
            g = _rb(jnp.dot(xs, wg_v[...], preferred_element_type=F32))
            g = _rb(g * _sigmoid(g))
            u = _rb(jnp.dot(xs, wu_v[...], preferred_element_type=F32))
            hh = (g * u).astype(BF)
            y = _rb(lax.dot_general(hh, wdt_v[...], NT, preferred_element_type=F32))
            y = _rb(y * _rb(_sigmoid(val)))
            yt = y.T
            for c in range(C):
                yb_v[c] = jnp.broadcast_to(yt[:, c:c + 1], (D, 128))
            idx_v[...] = jnp.broadcast_to(idx, (C, 128))

        def qk(u, s_ref, m_ref):
            h = lax.shift_right_logical(u, LOG_NQ)
            q2 = qo_v[u]
            m_acc = None
            for j in range(S // CK1):
                s = jnp.dot(k_v[h, j * CK1:(j + 1) * CK1, :], q2, preferred_element_type=F32)
                s_ref[j * CK1:(j + 1) * CK1, :] = s
                mm = jnp.max(s.reshape(CK1 // 8, 8, W), axis=0)
                m_acc = mm if m_acc is None else jnp.maximum(m_acc, mm)
            m_ref[...] = jnp.broadcast_to(jnp.max(m_acc, axis=0, keepdims=True), (8, W))

        def pv(u, s_ref, m_ref):
            h = lax.shift_right_logical(u, LOG_NQ)
            for c in range(W // PVW):
                sl = slice(c * PVW, (c + 1) * PVW)
                m = m_ref[0:1, sl]
                l_acc = jnp.zeros((8, PVW), F32)
                acc = jnp.zeros((DH, PVW), F32)
                for j in range(S // CK2):
                    p = jnp.exp2(s_ref[j * CK2:(j + 1) * CK2, sl] - m)
                    l_acc = l_acc + jnp.sum(p.reshape(CK2 // 8, 8, PVW), axis=0)
                    acc = acc + jnp.dot(vt_v[h, :, j * CK2:(j + 1) * CK2], p.astype(BF),
                                        preferred_element_type=F32)
                l = jnp.sum(l_acc, axis=0, keepdims=True)
                qo_v[u, :, sl] = (acc * (1.0 / l)).astype(BF)

        with jax.named_scope('kfwait'):
            for i in range(4):
                cp_f(i).wait()
            for h in range(HKV):
                cp_k(h).wait()
        with jax.named_scope('qk0_ffn'):
            qk(0, sa_v, ma_v)
            router_ffn()

        def p2_body(v, c):
            par = lax.bitwise_and(v, 1)

            @pl.when(par == 1)
            def _():
                qk(v, sb_v, mb_v)
                pv(v - 1, sa_v, ma_v)

            @pl.when(par == 0)
            def _():
                qk(v, sa_v, ma_v)
                pv(v - 1, sb_v, mb_v)
            return c
        with jax.named_scope('p2'):
            lax.fori_loop(1, U, p2_body, 0)
        with jax.named_scope('pvlast'):
            pv(U - 1, sb_v, mb_v)

        TPB = TQ // TB
        LOG_TPB = int(math.log2(TPB))

        def outproj(b, slot):
            i = lax.shift_right_logical(b, LOG_TPB) if not isinstance(b, int) else b // TPB
            t0 = (lax.bitwise_and(b, TPB - 1) if not isinstance(b, int) else b % TPB) * TB
            cols = []
            for h in range(HKV):
                for a in range(2):
                    off = a * TQ + t0
                    off = off if isinstance(off, int) else pl.multiple_of(off, 128)
                    cols.append(qo_v[h * NQ + i, :, pl.ds(off, TB)])
            rhs = jnp.concatenate(cols, axis=0)
            st_v[slot] = jnp.dot(wot_v[...], rhs, preferred_element_type=F32)

        def epilogue(b, slot):
            off = b * TB
            cols = pl.ds(off if isinstance(off, int) else pl.multiple_of(off, TB), TB)
            tok = (lax.broadcasted_iota(jnp.int32, (1, TB), 1) + b * TB).astype(F32)
            upd = jnp.zeros((D, TB), F32)
            for c in range(C):
                hit = tok == idx_v[c:c + 1, 0:1]
                yb = jnp.concatenate([yb_v[c]] * (TB // 128), axis=1)
                upd = jnp.where(hit, yb, upd)
            bo = _rb(xnt_v[:, cols].astype(F32) + upd)
            g = _rb(bo * _sigmoid(bo))
            os_v[slot] = (xt_v[:, cols].astype(F32) + _rb(_rb(st_v[slot]) * g)).astype(BF)

        with jax.named_scope('op0'):
            outproj(0, 0)

        def p3_body(b, c):
            slot = lax.bitwise_and(b, 1)
            prev = 1 - slot

            @pl.when(b >= 3)
            def _():
                cp_o(b - 3, prev).wait()
            epilogue(b - 1, prev)
            outproj(b, slot)
            cp_o(b - 1, prev).start()
            return c
        with jax.named_scope('p3'):
            lax.fori_loop(1, NB, p3_body, 0)
        last = (NB - 1) % 2
        cp_o(NB - 3, last).wait()
        with jax.named_scope('eplast'):
            epilogue(NB - 1, last)
        cp_o(NB - 1, last).start()
        cp_o(NB - 2, 1 - last).wait()
        cp_o(NB - 1, last).wait()

    scratch = [
        pltpu.VMEM((D, S), BF),
        pltpu.VMEM((D, S), BF),
        pltpu.VMEM((HKV, S, DH), BF),
        pltpu.VMEM((HKV, S, DH), BF),
        pltpu.VMEM((HKV, DH, S), BF),
        pltpu.VMEM((HKV, D, 256), BF),
        pltpu.VMEM((D, 2 * HKV * DH), BF),
        pltpu.VMEM((U, DH, W), BF),
        pltpu.VMEM((S, W), F32),
        pltpu.VMEM((S, W), F32),
        pltpu.VMEM((8, W), F32),
        pltpu.VMEM((8, W), F32),
        pltpu.VMEM((D, F), BF),
        pltpu.VMEM((D, F), BF),
        pltpu.VMEM((D, F), BF),
        pltpu.VMEM((C, D, 128), F32),
        pltpu.VMEM((C, 128), F32),
        pltpu.VMEM((2, D, TB), F32),
        pltpu.VMEM((2, D, TB), BF),
        pltpu.SemaphoreType.DMA((1,)),
        pltpu.SemaphoreType.DMA((HKV,)),
        pltpu.SemaphoreType.DMA((HKV,)),
        pltpu.SemaphoreType.DMA((HKV,)),
        pltpu.SemaphoreType.DMA((4,)),
        pltpu.SemaphoreType.DMA((2,)),
    ]

    def fn(A_x, A_k_cache, A_v_cache, A_wq, A_wo, B_x, B_w_r, B_w_gate, B_w_up, B_w_down):
        any_spec = pl.BlockSpec(memory_space=pl.ANY)
        out_t = pl.pallas_call(
            kernel,
            in_specs=[any_spec] * 8 + [pl.BlockSpec(memory_space=pltpu.VMEM)],
            out_specs=any_spec,
            out_shape=jax.ShapeDtypeStruct((D, S), BF),
            scratch_shapes=scratch,
            compiler_params=pltpu.CompilerParams(vmem_limit_bytes=120 * 1024 * 1024),
        )(A_x.reshape(S, D).T, A_k_cache.reshape(HKV, S, DH), A_v_cache.reshape(HKV, S, DH),
          A_wq, A_wo.T, B_w_gate, B_w_up, B_w_down.T, B_w_r.reshape(1, D))
        return out_t.T.reshape(1, S, D)

    return fn


_kernel_fn = make_kernel()


@jax.jit
def pallas_recurrent_scan__gqa_block_cached__moe_arch_mod__prompt_kernel(
    A_x: jax.Array,
    A_k_cache: jax.Array,
    A_v_cache: jax.Array,
    A_wq: jax.Array,
    A_wo: jax.Array,
    B_x: jax.Array,
    B_w_r: jax.Array,
    B_w_gate: jax.Array,
    B_w_up: jax.Array,
    B_w_down: jax.Array,
):
    return _kernel_fn(A_x, A_k_cache, A_v_cache, A_wq, A_wo, B_x, B_w_r, B_w_gate, B_w_up, B_w_down)
```

```python
import functools
import math

import jax
import jax.numpy as jnp
from jax import lax
from jax.experimental import pallas as pl
from jax.experimental.pallas import tpu as pltpu

S = 2048
D = 576
HKV = 16
DH = 128
F = 4608
C = 8
EPS = 1e-5

NT = (((1,), (1,)), ((), ()))
BF = jnp.bfloat16
F32 = jnp.float32


def _rb(x):
    return x.astype(BF).astype(F32)


def _sigmoid(x):
    return 1.0 / (1.0 + jnp.exp(-x))


def make_kernel(TQ=512, TB=512, SUB=256, CK1=256, CK2=128, PVW=512, LNB=256, XA=3, ORD=1, UPD=1, PIPE=1, LNFIRST=True):
    NQ = S // TQ
    LOG_NQ = int(math.log2(NQ))
    W = 2 * TQ
    U = HKV * NQ
    NB = S // TB
    NLN = S // LNB
    QSCALE = (DH ** -0.5) * math.log2(math.e)

    def kernel(xt_hbm, k_hbm, v_hbm, wq_hbm, wot_hbm, wg_hbm, wu_hbm, wdt_hbm, wr_ref,
               o_hbm,
               xt_v, xnt_v, k_v, v_v, vt_v, wq_v, wqt_v, wot_v, qo_v,
               sa_v, sb_v, ma_v, mb_v, wg_v, wu_v, wdt_v, os_v, r_v, yt_v, idx_v,
               sem_x, sem_wq, sem_v, sem_k, sem_f, sem_o):

        def cp_x(b):
            cols = pl.ds(b * LNB, LNB)
            return pltpu.make_async_copy(xt_hbm.at[:, cols], xt_v.at[:, cols], sem_x.at[b])

        def cp_wq(h):
            off = h * 256 if isinstance(h, int) else pl.multiple_of(h * 256, 256)
            return pltpu.make_async_copy(wq_hbm.at[:, pl.ds(off, 256)], wq_v.at[h], sem_wq.at[h])

        def cp_v(h):
            return pltpu.make_async_copy(v_hbm.at[h], v_v.at[h], sem_v.at[h])

        def cp_k(h):
            return pltpu.make_async_copy(k_hbm.at[h], k_v.at[h], sem_k.at[h])

        def cp_f(i):
            if i == 6:
                return pltpu.make_async_copy(wot_hbm, wot_v, sem_f.at[i])
            src, dst = ((wg_hbm, wg_v), (wu_hbm, wu_v), (wdt_hbm, wdt_v))[i // 2]
            cols = pl.ds((i % 2) * (F // 2), F // 2)
            return pltpu.make_async_copy(src.at[:, cols], dst.at[:, cols], sem_f.at[i])

        def cp_o(b, slot):
            return pltpu.make_async_copy(
                os_v.at[slot], o_hbm.at[:, pl.ds(pl.multiple_of(b * TB, TB), TB)], sem_o.at[slot])

        def layernorm(b):
            cols = slice(b * LNB, (b + 1) * LNB)
            x = xt_v[:, cols].astype(F32)
            mean = jnp.sum(x, axis=0, keepdims=True) * (1.0 / D)
            xc = x - mean
            var = jnp.sum(xc * xc, axis=0, keepdims=True) * (1.0 / D)
            den = _rb(jnp.sqrt(_rb(_rb(var) + EPS)))
            xn = (_rb(x - _rb(mean)) * (1.0 / den)).astype(BF)
            xnt_v[:, cols] = xn
            return xn

        def store_q(h, qt, c0, n):
            qt = (qt * QSCALE).astype(BF)
            step = min(n, TQ)
            for o in range(0, n, step):
                i, t0 = (c0 + o) // TQ, (c0 + o) % TQ
                for a in range(2):
                    qo_v[h * NQ + i, :, a * TQ + t0:a * TQ + t0 + step] = qt[a * DH:(a + 1) * DH, o:o + step]

        with jax.named_scope('p1first'):
            cp_x(0).start()
            cp_wq(0).start()
            cp_wq(1).start()
            for b in range(1, XA):
                cp_x(b).start()
            with jax.named_scope('w1'):
                cp_x(0).wait()
                for b in range(XA, NLN):
                    cp_x(b).start()
                if PIPE == 0:
                    cp_wq(0).wait()
                    cp_wq(1).wait()
            xn = layernorm(0)
            if PIPE > 0:
                cp_wq(0).wait()
                cp_wq(1).wait()
            wqt = [wq_v[h].T for h in range(2)]
            for b in range(NLN):
                if b + 1 < NLN:
                    if b + 1 == NLN - 1:
                        for h in range(2, 5):
                            cp_wq(h).start()
                        for h in range(4):
                            cp_v(h).start()
                    cp_x(b + 1).wait()
                if LNFIRST and b + 1 < NLN:
                    xn_next = layernorm(b + 1)
                for h in range(2):
                    store_q(h, jnp.dot(wqt[h], xn, preferred_element_type=F32), b * LNB, LNB)
                if not LNFIRST and b + 1 < NLN:
                    xn_next = layernorm(b + 1)
                xn = xn_next
            wr8 = jnp.broadcast_to(wr_ref[...], (C, D))
            r_v[...] = _rb(jnp.dot(wr8, xnt_v[...], preferred_element_type=F32))
            cp_wq(2).wait()
            wqt_v[...] = wq_v[2].T

        NT1 = HKV // 2
        def p1_body(t, c):
            h0 = 2 * t
            h2 = jnp.minimum(h0 + 2, HKV - 1)
            @pl.when(t < NT1 - 2)
            def _():
                cp_wq(h0 + 4).start()

            @pl.when(t < NT1 - 1)
            def _():
                cp_wq(h0 + 3).start()
                cp_v(h0 + 2).start()
                cp_v(h0 + 3).start()
            for i in range(6):
                @pl.when(t == 1 + i)
                def _():
                    cp_f(i).start()

            @pl.when(t == NT1 - 1)
            def _():
                for h in range(4):
                    cp_k(h).start()

            @pl.when(t < NT1 - 1)
            def _():
                cp_wq(h0 + 2).wait()
            cp_wq(h0 + 1).wait()
            cp_v(h0).wait()
            cp_v(h0 + 1).wait()
            store_q(h0, jnp.dot(wqt_v[...], xnt_v[...], preferred_element_type=F32), 0, S)
            store_q(h0 + 1, jnp.dot(wq_v[h0 + 1].T, xnt_v[...], preferred_element_type=F32), 0, S)
            wqt_v[...] = wq_v[h2].T
            vt_v[h0] = v_v[h0].T
            vt_v[h0 + 1] = v_v[h0 + 1].T
            return c
        with jax.named_scope('p1'):
            lax.fori_loop(1, NT1, p1_body, 0)

        def router_ffn():
            r = r_v[...]
            tok = lax.broadcasted_iota(jnp.int32, (C, S), 1).astype(F32)
            row = lax.broadcasted_iota(jnp.int32, (C, 1), 0)
            idx = jnp.zeros((C, 1), F32)
            val = jnp.zeros((C, 1), F32)
            for c in range(C):
                mx = jnp.max(r, axis=1, keepdims=True)
                ix = jnp.min(jnp.where(r == mx, tok, float(S)), axis=1, keepdims=True)
                r = jnp.where(tok == ix, -jnp.inf, r)
                idx = jnp.where(row == c, ix, idx)
                val = jnp.where(row == c, mx, val)
            onehot = jnp.where(tok == idx, 1.0, 0.0).astype(BF)
            xs = lax.dot_general(onehot, xnt_v[...], NT, preferred_element_type=F32).astype(BF)
            g = _rb(jnp.dot(xs, wg_v[...], preferred_element_type=F32))
            g = _rb(g * _sigmoid(g))
            u = _rb(jnp.dot(xs, wu_v[...], preferred_element_type=F32))
            hh = (g * u).astype(BF)
            y = _rb(lax.dot_general(hh, wdt_v[...], NT, preferred_element_type=F32))
            y = _rb(y * _rb(_sigmoid(val)))
            yt_v[...] = y.T
            idx_v[...] = jnp.broadcast_to(jnp.minimum(idx, float(S - 1)).astype(jnp.int32), (C, 128))

        def scatter_update():
            lane = lax.broadcasted_iota(jnp.int32, (1, 128), 1)
            for c in range(C):
                t = idx_v[c, 0]
                cols = pl.ds(pl.multiple_of(lax.shift_right_logical(t, 7) * 128, 128), 128)
                xb = xnt_v[:, cols].astype(F32)
                hit = lane == lax.bitwise_and(t, 127)
                xnt_v[:, cols] = jnp.where(hit, xb + yt_v[:, c:c + 1], xb).astype(BF)

        def qk(u, s_ref, m_ref):
            h = lax.shift_right_logical(u, LOG_NQ)
            q2 = qo_v[u]
            m_acc = None
            for j in range(S // CK1):
                s = jnp.dot(k_v[h, j * CK1:(j + 1) * CK1, :], q2, preferred_element_type=F32)
                s_ref[j * CK1:(j + 1) * CK1, :] = s
                mm = jnp.max(s.reshape(CK1 // 8, 8, W), axis=0)
                m_acc = mm if m_acc is None else jnp.maximum(m_acc, mm)
            m_ref[...] = jnp.broadcast_to(jnp.max(m_acc, axis=0, keepdims=True), (8, W))

        def pv(u, s_ref, m_ref):
            h = lax.shift_right_logical(u, LOG_NQ)
            for c in range(W // PVW):
                sl = slice(c * PVW, (c + 1) * PVW)
                m = m_ref[0:1, sl]
                l_acc = jnp.zeros((8, PVW), F32)
                acc = jnp.zeros((DH, PVW), F32)
                for j in range(S // CK2):
                    p = jnp.exp2(s_ref[j * CK2:(j + 1) * CK2, sl] - m)
                    l_acc = l_acc + jnp.sum(p.reshape(CK2 // 8, 8, PVW), axis=0)
                    acc = acc + jnp.dot(vt_v[h, :, j * CK2:(j + 1) * CK2], p.astype(BF),
                                        preferred_element_type=F32)
                l = jnp.sum(l_acc, axis=0, keepdims=True)
                qo_v[u, :, sl] = (acc * (1.0 / l)).astype(BF)

        for h in range(4, HKV):
            cp_k(h).start()
        cp_f(6).start()
        with jax.named_scope('kfwait'):
            for i in range(6):
                cp_f(i).wait()
            cp_k(0).wait()
            cp_v(0).wait()
            cp_v(1).wait()
        with jax.named_scope('qk0_ffn'):
            if ORD == 0:
                router_ffn()
            qk(0, sa_v, ma_v)
            vt_v[0] = v_v[0].T
            vt_v[1] = v_v[1].T
            if ORD == 1:
                router_ffn()
            if UPD == 0:
                scatter_update()

        def p2_body(v, c):
            par = lax.bitwise_and(v, 1)

            @pl.when(lax.bitwise_and(v, NQ - 1) == 0)
            def _():
                cp_k(lax.shift_right_logical(v, LOG_NQ)).wait()

            @pl.when(par == 1)
            def _():
                qk(v, sb_v, mb_v)
                pv(v - 1, sa_v, ma_v)

            @pl.when(par == 0)
            def _():
                qk(v, sa_v, ma_v)
                pv(v - 1, sb_v, mb_v)
            return c
        with jax.named_scope('p2'):
            lax.fori_loop(1, U, p2_body, 0)
        with jax.named_scope('pvlast'):
            if UPD == 1:
                scatter_update()
            pv(U - 1, sb_v, mb_v)
            if UPD == 2:
                scatter_update()

        def p3_block(b, slot):
            for sub in range(TB // SUB):
                tok0 = b * TB + sub * SUB
                i = lax.shift_right_logical(tok0, int(math.log2(TQ)))
                t0 = lax.bitwise_and(tok0, TQ - 1)
                parts = []
                for h in range(HKV):
                    for a in range(2):
                        parts.append(qo_v[h * NQ + i, :, pl.ds(pl.multiple_of(a * TQ + t0, 128), SUB)])
                rhs = jnp.concatenate(parts, axis=0)
                s_t = jnp.dot(wot_v[...], rhs, preferred_element_type=F32)
                cols = pl.ds(pl.multiple_of(tok0, 128), SUB)
                bo = xnt_v[:, cols].astype(F32)
                g = bo * _sigmoid(bo)
                os_v[slot, :, sub * SUB:(sub + 1) * SUB] = (xt_v[:, cols].astype(F32) + s_t * g).astype(BF)

        def p3_body(b, c):
            slot = lax.bitwise_and(b, 1)

            @pl.when(b >= 2)
            def _():
                cp_o(b - 2, slot).wait()
            p3_block(b, slot)
            cp_o(b, slot).start()
            return c
        cp_f(6).wait()
        with jax.named_scope('p3'):
            lax.fori_loop(0, NB, p3_body, 0)
        cp_o(NB - 2, (NB - 2) % 2).wait()
        cp_o(NB - 1, (NB - 1) % 2).wait()

    scratch = [
        pltpu.VMEM((D, S), BF),
        pltpu.VMEM((D, S), BF),
        pltpu.VMEM((HKV, S, DH), BF),
        pltpu.VMEM((HKV, S, DH), BF),
        pltpu.VMEM((HKV, DH, S), BF),
        pltpu.VMEM((HKV, D, 256), BF),
        pltpu.VMEM((256, D), BF),
        pltpu.VMEM((D, 2 * HKV * DH), BF),
        pltpu.VMEM((U, DH, W), BF),
        pltpu.VMEM((S, W), F32),
        pltpu.VMEM((S, W), F32),
        pltpu.VMEM((8, W), F32),
        pltpu.VMEM((8, W), F32),
        pltpu.VMEM((D, F), BF),
        pltpu.VMEM((D, F), BF),
        pltpu.VMEM((D, F), BF),
        pltpu.VMEM((2, D, TB), BF),
        pltpu.VMEM((C, S), F32),
        pltpu.VMEM((D, C), F32),
        pltpu.VMEM((C, 128), jnp.int32),
        pltpu.SemaphoreType.DMA((NLN,)),
        pltpu.SemaphoreType.DMA((HKV,)),
        pltpu.SemaphoreType.DMA((HKV,)),
        pltpu.SemaphoreType.DMA((HKV,)),
        pltpu.SemaphoreType.DMA((7,)),
        pltpu.SemaphoreType.DMA((2,)),
    ]

    def fn(A_x, A_k_cache, A_v_cache, A_wq, A_wo, B_x, B_w_r, B_w_gate, B_w_up, B_w_down):
        any_spec = pl.BlockSpec(memory_space=pl.ANY)
        out_t = pl.pallas_call(
            kernel,
            in_specs=[any_spec] * 8 + [pl.BlockSpec(memory_space=pltpu.VMEM)],
            out_specs=any_spec,
            out_shape=jax.ShapeDtypeStruct((D, S), BF),
            scratch_shapes=scratch,
            compiler_params=pltpu.CompilerParams(vmem_limit_bytes=126 * 1024 * 1024),
        )(A_x.reshape(S, D).T, A_k_cache.reshape(HKV, S, DH), A_v_cache.reshape(HKV, S, DH),
          A_wq, A_wo.T, B_w_gate, B_w_up, B_w_down.T, B_w_r.reshape(1, D))
        return out_t.T.reshape(1, S, D)

    return fn


_kernel_fn = make_kernel(TQ=1024, PVW=2048, XA=2, CK1=1024, CK2=256)


@jax.jit
def pallas_recurrent_scan__gqa_block_cached__moe_arch_mod__prompt_kernel(
    A_x: jax.Array,
    A_k_cache: jax.Array,
    A_v_cache: jax.Array,
    A_wq: jax.Array,
    A_wo: jax.Array,
    B_x: jax.Array,
    B_w_r: jax.Array,
    B_w_gate: jax.Array,
    B_w_up: jax.Array,
    B_w_down: jax.Array,
):
    return _kernel_fn(A_x, A_k_cache, A_v_cache, A_wq, A_wo, B_x, B_w_r, B_w_gate, B_w_up, B_w_down)
```

```python
import math

import jax
import jax.numpy as jnp
from jax import lax
from jax.experimental import pallas as pl
from jax.experimental.pallas import tpu as pltpu

S = 2048
D = 576
HKV = 16
DH = 128
F = 4608
C = 8
EPS = 1e-5

TQ = 1024
NQ = S // TQ
W = 2 * TQ
U = HKV * NQ
CK1 = 1024
CK2 = 256
LNB = 256
NLN = S // LNB
XW = (0, 1, 2, 4)
TB = 512
SUB = 128
NB = S // TB
NSUB = TB // SUB
NT1 = HKV // 2
QSCALE = (DH ** -0.5) * math.log2(math.e)

NT = (((1,), (1,)), ((), ()))
BF = jnp.bfloat16
F32 = jnp.float32


def _rb(x):
    return x.astype(BF).astype(F32)


def _sigmoid(x):
    return 1.0 / (1.0 + jnp.exp(-x))


def _kernel(xt_hbm, k_hbm, v_hbm, wq_hbm, wot_hbm, wg_hbm, wu_hbm, wdt_hbm, wr_ref,
            o_hbm,
            xt_v, xnt_v, k_v, v_v, vt_v, wq_v, wqt_v, wot_v, qo_v,
            sa_v, sb_v, ma_v, mb_v, wg_v, wu_v, wdt_v, os_v, r_v, yt_v, idx_s,
            sem_x, sem_wq, sem_v, sem_k, sem_f, sem_o):

    def cp_x(b):
        cols = pl.ds(b * LNB, LNB)
        return pltpu.make_async_copy(xt_hbm.at[:, cols], xt_v.at[:, cols], sem_x.at[b])

    def cp_wq(h):
        off = h * 256 if isinstance(h, int) else pl.multiple_of(h * 256, 256)
        return pltpu.make_async_copy(wq_hbm.at[:, pl.ds(off, 256)], wq_v.at[h], sem_wq.at[h])

    def cp_v(h):
        return pltpu.make_async_copy(v_hbm.at[h], v_v.at[h], sem_v.at[h])

    def cp_k(h):
        return pltpu.make_async_copy(k_hbm.at[h], k_v.at[h], sem_k.at[h])

    def cp_f(i):
        if i == 6:
            return pltpu.make_async_copy(wot_hbm, wot_v, sem_f.at[i])
        src, dst = ((wg_hbm, wg_v), (wu_hbm, wu_v), (wdt_hbm, wdt_v))[i // 2]
        cols = pl.ds((i % 2) * (F // 2), F // 2)
        return pltpu.make_async_copy(src.at[:, cols], dst.at[:, cols], sem_f.at[i])

    def cp_o(b, slot, sub):
        off = b * TB + sub * SUB
        off = off if isinstance(off, int) else pl.multiple_of(off, SUB)
        return pltpu.make_async_copy(
            os_v.at[slot, sub], o_hbm.at[:, pl.ds(off, SUB)], sem_o.at[slot * NSUB + sub])

    def layernorm(b):
        cols = slice(b * LNB, (b + 1) * LNB)
        x = xt_v[:, cols].astype(F32)
        mean = jnp.sum(x, axis=0, keepdims=True) * (1.0 / D)
        xc = x - mean
        var = jnp.sum(xc * xc, axis=0, keepdims=True) * (1.0 / D)
        den = _rb(jnp.sqrt(_rb(_rb(var) + EPS)))
        xn = (_rb(x - _rb(mean)) * (1.0 / den)).astype(BF)
        xnt_v[:, cols] = xn
        return xn

    def store_q(h, qt, c0, n):
        qt = (qt * QSCALE).astype(BF)
        step = min(n, TQ)
        for o in range(0, n, step):
            i, t0 = (c0 + o) // TQ, (c0 + o) % TQ
            for a in range(2):
                qo_v[h * NQ + i, :, a * TQ + t0:a * TQ + t0 + step] = qt[a * DH:(a + 1) * DH, o:o + step]

    with jax.named_scope('p1first'):
        cp_wq(0).start()
        cp_x(0).start()
        cp_wq(1).start()
        cp_x(1).start()
        wr16 = jnp.broadcast_to(wr_ref[...].reshape(1, D), (16, D))
        cp_wq(0).wait()
        wqt_v[...] = wq_v[0].T
        cp_x(0).wait()
        for b in range(2, NLN):
            cp_x(b).start()
        cp_wq(2).start()
        xn = layernorm(0)
        wqt = [wqt_v[...], None]
        store_q(0, jnp.dot(wqt[0], xn, preferred_element_type=F32), 0, LNB)
        for b in range(NLN):
            if b in XW:
                nxt = min([w for w in XW if w > b] + [NLN - 1])
                if b == 0:
                    cp_wq(1).wait()
                for bb in range(b + 1, nxt + 1):
                    if bb == NLN - 1:
                        for h in range(3, 5):
                            cp_wq(h).start()
                        for h in range(4):
                            cp_v(h).start()
                        cp_wq(2).wait()
                    cp_x(bb).wait()
            if b == 0:
                wqt[1] = jnp.concatenate([wq_v[1].T, wr16], axis=0)
            if b + 1 < NLN:
                xn_next = layernorm(b + 1)
            for h in range(2):
                if b == 0 and h == 0:
                    continue
                qt = jnp.dot(wqt[h], xn, preferred_element_type=F32)
                if h == 1:
                    r_v[:, b * LNB:(b + 1) * LNB] = _rb(qt[256:256 + C, :])
                    qt = qt[0:256, :]
                store_q(h, qt, b * LNB, LNB)
            xn = xn_next
        wqt_v[...] = wq_v[2].T
        cp_wq(5).start()
        cp_wq(6).start()
        cp_v(4).start()
        cp_v(5).start()

    def p1_body(t, c):
        h0 = 2 * t
        h2 = jnp.minimum(h0 + 2, HKV - 1)

        @pl.when(t < NT1 - 1)
        def _():
            cp_wq(h0 + 2).wait()
        cp_wq(h0 + 1).wait()
        cp_v(h0).wait()
        cp_v(h0 + 1).wait()
        store_q(h0, jnp.dot(wqt_v[...], xnt_v[...], preferred_element_type=F32), 0, S)
        store_q(h0 + 1, jnp.dot(wq_v[h0 + 1].T, xnt_v[...], preferred_element_type=F32), 0, S)
        wqt_v[...] = wq_v[h2].T
        vt_v[h0] = v_v[h0].T
        vt_v[h0 + 1] = v_v[h0 + 1].T

        @pl.when(t < NT1 - 2)
        def _():
            cp_wq(h0 + 5).start()
            cp_v(h0 + 4).start()
            cp_v(h0 + 5).start()

        @pl.when(t < NT1 - 3)
        def _():
            cp_wq(h0 + 6).start()
        for i in range(6):
            @pl.when(t == 1 + i)
            def _():
                cp_f(i).start()
        for g in range(2):
            @pl.when(t == NT1 - 3 + g)
            def _():
                cp_k(2 * g).start()
                cp_k(2 * g + 1).start()
        return c
    with jax.named_scope('p1'):
        lax.fori_loop(1, NT1, p1_body, 0)

    def router_ffn():
        r = r_v[...]
        tok = lax.broadcasted_iota(jnp.int32, (C, S), 1).astype(F32)
        row = lax.broadcasted_iota(jnp.int32, (C, 1), 0)
        idx = jnp.zeros((C, 1), F32)
        val = jnp.zeros((C, 1), F32)
        for c in range(C):
            mx = jnp.max(r, axis=1, keepdims=True)
            ix = jnp.min(jnp.where(r == mx, tok, float(S)), axis=1, keepdims=True)
            r = jnp.where(tok == ix, -jnp.inf, r)
            idx = jnp.where(row == c, ix, idx)
            val = jnp.where(row == c, mx, val)
        idx_i = jnp.minimum(idx, float(S - 1)).astype(jnp.int32)
        for c in range(C):
            idx_s[c] = idx_i[c, 0]
        onehot = jnp.where(tok == idx, 1.0, 0.0).astype(BF)
        xs = lax.dot_general(onehot, xnt_v[...], NT, preferred_element_type=F32).astype(BF)
        g = _rb(jnp.dot(xs, wg_v[...], preferred_element_type=F32))
        g = _rb(g * _sigmoid(g))
        u = _rb(jnp.dot(xs, wu_v[...], preferred_element_type=F32))
        hh = (g * u).astype(BF)
        y = _rb(lax.dot_general(hh, wdt_v[...], NT, preferred_element_type=F32))
        y = _rb(y * _rb(_sigmoid(val)))
        yt_v[...] = y.T

    def scatter_update():
        lane = lax.broadcasted_iota(jnp.int32, (1, 128), 1)
        for c in range(C):
            t = idx_s[c]
            cols = pl.ds(pl.multiple_of(lax.shift_right_logical(t, 7) * 128, 128), 128)
            xb = xnt_v[:, cols].astype(F32)
            hit = lane == lax.bitwise_and(t, 127)
            xnt_v[:, cols] = jnp.where(hit, xb + yt_v[:, c:c + 1], xb).astype(BF)

    def head(u):
        return u // NQ if isinstance(u, int) else lax.shift_right_logical(u, int(math.log2(NQ)))

    def qk(u, s_ref, m_ref):
        h = head(u)
        q2 = qo_v[u]
        m_acc = None
        for j in range(S // CK1):
            s = jnp.dot(k_v[h, j * CK1:(j + 1) * CK1, :], q2, preferred_element_type=F32)
            s_ref[j * CK1:(j + 1) * CK1, :] = s
            mm = jnp.max(s.reshape(CK1 // 8, 8, W), axis=0)
            m_acc = mm if m_acc is None else jnp.maximum(m_acc, mm)
        m_ref[...] = jnp.broadcast_to(jnp.max(m_acc, axis=0, keepdims=True), (8, W))

    def pv(u, s_ref, m_ref):
        h = head(u)
        m = m_ref[0:1, :]
        l_acc = jnp.zeros((8, W), F32)
        acc = jnp.zeros((DH, W), F32)
        for j in range(S // CK2):
            p = jnp.exp2(s_ref[j * CK2:(j + 1) * CK2, :] - m)
            l_acc = l_acc + jnp.sum(p.reshape(CK2 // 8, 8, W), axis=0)
            acc = acc + jnp.dot(vt_v[h, :, j * CK2:(j + 1) * CK2], p.astype(BF), preferred_element_type=F32)
        l = jnp.sum(l_acc, axis=0, keepdims=True)
        qo_v[u] = (acc * (1.0 / l)).astype(BF)

    for h in range(4, HKV):
        cp_k(h).start()
    cp_f(6).start()
    for i in range(6):
        cp_f(i).wait()
    cp_k(0).wait()
    cp_v(0).wait()
    cp_v(1).wait()
    with jax.named_scope('qk0_ffn'):
        qk(0, sa_v, ma_v)
        vt_v[0] = v_v[0].T
        vt_v[1] = v_v[1].T
        router_ffn()

    def p2_body(v, c):
        par = lax.bitwise_and(v, 1)

        @pl.when(lax.bitwise_and(v, NQ - 1) == 0)
        def _():
            cp_k(head(v)).wait()

        @pl.when(par == 1)
        def _():
            qk(v, sb_v, mb_v)
            pv(v - 1, sa_v, ma_v)

        @pl.when(par == 0)
        def _():
            qk(v, sa_v, ma_v)
            pv(v - 1, sb_v, mb_v)
        return c
    with jax.named_scope('p2'):
        lax.fori_loop(1, U, p2_body, 0)
    with jax.named_scope('pvlast'):
        scatter_update()
        pv(U - 1, sb_v, mb_v)

    def p3_body(b, c):
        slot = lax.bitwise_and(b, 1)

        @pl.when(b >= 2)
        def _():
            for sub in range(NSUB):
                cp_o(b - 2, slot, sub).wait()
        for sub in range(NSUB):
            tok0 = b * TB + sub * SUB
            i = lax.shift_right_logical(tok0, int(math.log2(TQ)))
            t0 = lax.bitwise_and(tok0, TQ - 1)
            parts = []
            for h in range(HKV):
                for a in range(2):
                    parts.append(qo_v[h * NQ + i, :, pl.ds(pl.multiple_of(a * TQ + t0, 128), SUB)])
            rhs = jnp.concatenate(parts, axis=0)
            s_t = jnp.dot(wot_v[...], rhs, preferred_element_type=F32)
            cols = pl.ds(pl.multiple_of(tok0, 128), SUB)
            bo = xnt_v[:, cols].astype(F32)
            g = bo * _sigmoid(bo)
            os_v[slot, sub] = (xt_v[:, cols].astype(F32) + s_t * g).astype(BF)
            cp_o(b, slot, sub).start()
        return c
    cp_f(6).wait()
    with jax.named_scope('p3'):
        lax.fori_loop(0, NB, p3_body, 0)
    for bb in (NB - 2, NB - 1):
        for sub in range(NSUB):
            cp_o(bb, bb % 2, sub).wait()


_SCRATCH = [
    pltpu.VMEM((D, S), BF),
    pltpu.VMEM((D, S), BF),
    pltpu.VMEM((HKV, S, DH), BF),
    pltpu.VMEM((HKV, S, DH), BF),
    pltpu.VMEM((HKV, DH, S), BF),
    pltpu.VMEM((HKV, D, 256), BF),
    pltpu.VMEM((256, D), BF),
    pltpu.VMEM((D, 2 * HKV * DH), BF),
    pltpu.VMEM((U, DH, W), BF),
    pltpu.VMEM((S, W), F32),
    pltpu.VMEM((S, W), F32),
    pltpu.VMEM((8, W), F32),
    pltpu.VMEM((8, W), F32),
    pltpu.VMEM((D, F), BF),
    pltpu.VMEM((D, F), BF),
    pltpu.VMEM((D, F), BF),
    pltpu.VMEM((2, NSUB, D, SUB), BF),
    pltpu.VMEM((C, S), F32),
    pltpu.VMEM((D, C), F32),
    pltpu.SMEM((C,), jnp.int32),
    pltpu.SemaphoreType.DMA((NLN,)),
    pltpu.SemaphoreType.DMA((HKV,)),
    pltpu.SemaphoreType.DMA((HKV,)),
    pltpu.SemaphoreType.DMA((HKV,)),
    pltpu.SemaphoreType.DMA((7,)),
    pltpu.SemaphoreType.DMA((2 * NSUB,)),
]


def _run(A_x, A_k_cache, A_v_cache, A_wq, A_wo, B_x, B_w_r, B_w_gate, B_w_up, B_w_down):
    any_spec = pl.BlockSpec(memory_space=pl.ANY)
    out_t = pl.pallas_call(
        _kernel,
        in_specs=[any_spec] * 8 + [pl.BlockSpec(memory_space=pltpu.VMEM)],
        out_specs=any_spec,
        out_shape=jax.ShapeDtypeStruct((D, S), BF),
        scratch_shapes=_SCRATCH,
        compiler_params=pltpu.CompilerParams(vmem_limit_bytes=126 * 1024 * 1024,
                                             disable_bounds_checks=True),
    )(A_x.reshape(S, D).T, A_k_cache.reshape(HKV, S, DH), A_v_cache.reshape(HKV, S, DH),
      A_wq, A_wo.T, B_w_gate, B_w_up, B_w_down.T, B_w_r)
    return out_t.T.reshape(1, S, D)


@jax.jit
def pallas_recurrent_scan__gqa_block_cached__moe_arch_mod__prompt_kernel(
    A_x: jax.Array,
    A_k_cache: jax.Array,
    A_v_cache: jax.Array,
    A_wq: jax.Array,
    A_wo: jax.Array,
    B_x: jax.Array,
    B_w_r: jax.Array,
    B_w_gate: jax.Array,
    B_w_up: jax.Array,
    B_w_down: jax.Array,
):
    return _run(A_x, A_k_cache, A_v_cache, A_wq, A_wo, B_x, B_w_r, B_w_gate, B_w_up, B_w_down)
```

```python
import math

import jax
import jax.numpy as jnp
from jax import lax
from jax.experimental import pallas as pl
from jax.experimental.pallas import tpu as pltpu

S = 2048
D = 576
HKV = 16
DH = 128
F = 4608
C = 8
EPS = 1e-5

TQ = 1024
NQ = S // TQ
W = 2 * TQ
U = HKV * NQ
CK1 = 1024
CK2 = 256
LNB = 128
NLN = S // LNB
XW = (0, 2, 4, 8)
TB = 512
SUB = 128
NB = S // TB
NSUB = TB // SUB
NT1 = HKV // 2
QSCALE = (DH ** -0.5) * math.log2(math.e)

NT = (((1,), (1,)), ((), ()))
BF = jnp.bfloat16
F32 = jnp.float32


def _rb(x):
    return x.astype(BF).astype(F32)


def _sigmoid(x):
    return 1.0 / (1.0 + jnp.exp(-x))


def _kernel(xt_hbm, k_hbm, v_hbm, wq_hbm, wot_hbm, wg_hbm, wu_hbm, wdt_hbm, wr_ref,
            o_hbm,
            xt_v, xnt_v, k_v, v_v, vt_v, wq_v, wqt_v, wot_v, qo_v,
            sa_v, sb_v, ma_v, mb_v, wg_v, wu_v, wdt_v, os_v, r_v, yt_v, idx_s,
            sem_x, sem_wq, sem_v, sem_k, sem_f, sem_o):

    def cp_x(b):
        cols = pl.ds(b * LNB, LNB)
        return pltpu.make_async_copy(xt_hbm.at[:, cols], xt_v.at[:, cols], sem_x.at[b])

    def cp_wq(h):
        off = h * 256 if isinstance(h, int) else pl.multiple_of(h * 256, 256)
        return pltpu.make_async_copy(wq_hbm.at[:, pl.ds(off, 256)], wq_v.at[h], sem_wq.at[h])

    def cp_v(h):
        return pltpu.make_async_copy(v_hbm.at[h], v_v.at[h], sem_v.at[h])

    def cp_k(h):
        return pltpu.make_async_copy(k_hbm.at[h], k_v.at[h], sem_k.at[h])

    def cp_f(i):
        if i == 6:
            return pltpu.make_async_copy(wot_hbm, wot_v, sem_f.at[i])
        src, dst = ((wg_hbm, wg_v), (wu_hbm, wu_v), (wdt_hbm, wdt_v))[i // 2]
        cols = pl.ds((i % 2) * (F // 2), F // 2)
        return pltpu.make_async_copy(src.at[:, cols], dst.at[:, cols], sem_f.at[i])

    def cp_o(b, sub):
        off = b * TB + sub * SUB
        off = off if isinstance(off, int) else pl.multiple_of(off, SUB)
        return pltpu.make_async_copy(
            os_v.at[b, sub], o_hbm.at[:, pl.ds(off, SUB)], sem_o.at[b * NSUB + sub])

    def layernorm(b):
        cols = slice(b * LNB, (b + 1) * LNB)
        x = xt_v[:, cols].astype(F32)
        mean = jnp.sum(x, axis=0, keepdims=True) * (1.0 / D)
        xc = x - mean
        var = jnp.sum(xc * xc, axis=0, keepdims=True) * (1.0 / D)
        den = _rb(jnp.sqrt(_rb(_rb(var) + EPS)))
        xn = (_rb(x - _rb(mean)) * (1.0 / den)).astype(BF)
        xnt_v[:, cols] = xn
        return xn

    def store_q(h, qt, c0, n):
        qt = (qt * QSCALE).astype(BF)
        step = min(n, TQ)
        for o in range(0, n, step):
            i, t0 = (c0 + o) // TQ, (c0 + o) % TQ
            for a in range(2):
                qo_v[h * NQ + i, :, a * TQ + t0:a * TQ + t0 + step] = qt[a * DH:(a + 1) * DH, o:o + step]

    with jax.named_scope('p1first'):
        cp_wq(0).start()
        cp_x(0).start()
        cp_wq(1).start()
        cp_x(1).start()
        wr16 = jnp.broadcast_to(wr_ref[...].reshape(1, D), (16, D))
        cp_wq(0).wait()
        wqt_v[...] = wq_v[0].T
        cp_x(0).wait()
        for b in range(2, NLN):
            cp_x(b).start()
        cp_wq(2).start()
        xn = layernorm(0)
        wqt = [wqt_v[...], None]
        store_q(0, jnp.dot(wqt[0], xn, preferred_element_type=F32), 0, LNB)
        for b in range(NLN):
            if b in XW:
                nxt = min([w for w in XW if w > b] + [NLN - 1])
                if b == 0:
                    cp_wq(1).wait()
                for bb in range(b + 1, nxt + 1):
                    if bb == NLN - 1:
                        for h in range(3, 5):
                            cp_wq(h).start()
                        for h in range(4):
                            cp_v(h).start()
                        cp_wq(2).wait()
                    cp_x(bb).wait()
            if b == 0:
                wqt[1] = jnp.concatenate([wq_v[1].T, wr16], axis=0)
            if b + 1 < NLN:
                xn_next = layernorm(b + 1)
            for h in range(2):
                if b == 0 and h == 0:
                    continue
                qt = jnp.dot(wqt[h], xn, preferred_element_type=F32)
                if h == 1:
                    r_v[:, b * LNB:(b + 1) * LNB] = _rb(qt[256:256 + C, :])
                    qt = qt[0:256, :]
                store_q(h, qt, b * LNB, LNB)
            xn = xn_next
        wqt_v[...] = wq_v[2].T
        cp_wq(5).start()
        cp_wq(6).start()
        cp_v(4).start()
        cp_v(5).start()

    def p1_body(t, c):
        h0 = 2 * t
        h2 = jnp.minimum(h0 + 2, HKV - 1)

        @pl.when(t < NT1 - 1)
        def _():
            cp_wq(h0 + 2).wait()
        cp_wq(h0 + 1).wait()
        cp_v(h0).wait()
        cp_v(h0 + 1).wait()
        store_q(h0, jnp.dot(wqt_v[...], xnt_v[...], preferred_element_type=F32), 0, S)
        store_q(h0 + 1, jnp.dot(wq_v[h0 + 1].T, xnt_v[...], preferred_element_type=F32), 0, S)
        wqt_v[...] = wq_v[h2].T
        vt_v[h0] = v_v[h0].T
        vt_v[h0 + 1] = v_v[h0 + 1].T

        @pl.when(t < NT1 - 2)
        def _():
            cp_wq(h0 + 5).start()
            cp_v(h0 + 4).start()
            cp_v(h0 + 5).start()

        @pl.when(t < NT1 - 3)
        def _():
            cp_wq(h0 + 6).start()
        for i in range(6):
            @pl.when(t == 1 + i)
            def _():
                cp_f(i).start()
        for g in range(2):
            @pl.when(t == NT1 - 3 + g)
            def _():
                cp_k(2 * g).start()
                cp_k(2 * g + 1).start()
        return c
    with jax.named_scope('p1'):
        lax.fori_loop(1, NT1, p1_body, 0)

    def router_ffn():
        r = r_v[...]
        tok = lax.broadcasted_iota(jnp.int32, (C, S), 1).astype(F32)
        row = lax.broadcasted_iota(jnp.int32, (C, 1), 0)
        idx = jnp.zeros((C, 1), F32)
        val = jnp.zeros((C, 1), F32)
        for c in range(C):
            mx = jnp.max(r, axis=1, keepdims=True)
            ix = jnp.min(jnp.where(r == mx, tok, float(S)), axis=1, keepdims=True)
            r = jnp.where(tok == ix, -jnp.inf, r)
            idx = jnp.where(row == c, ix, idx)
            val = jnp.where(row == c, mx, val)
        idx_i = jnp.minimum(idx, float(S - 1)).astype(jnp.int32)
        for c in range(C):
            idx_s[c] = idx_i[c, 0]
        onehot = jnp.where(tok == idx, 1.0, 0.0).astype(BF)
        xs = lax.dot_general(onehot, xnt_v[...], NT, preferred_element_type=F32).astype(BF)
        g = _rb(jnp.dot(xs, wg_v[...], preferred_element_type=F32))
        g = _rb(g * _sigmoid(g))
        u = _rb(jnp.dot(xs, wu_v[...], preferred_element_type=F32))
        hh = (g * u).astype(BF)
        y = _rb(lax.dot_general(hh, wdt_v[...], NT, preferred_element_type=F32))
        y = _rb(y * _rb(_sigmoid(val)))
        yt_v[...] = y.T

    def scatter_update():
        lane = lax.broadcasted_iota(jnp.int32, (1, 128), 1)
        for c in range(C):
            t = idx_s[c]
            cols = pl.ds(pl.multiple_of(lax.shift_right_logical(t, 7) * 128, 128), 128)
            xb = xnt_v[:, cols].astype(F32)
            hit = lane == lax.bitwise_and(t, 127)
            xnt_v[:, cols] = jnp.where(hit, xb + yt_v[:, c:c + 1], xb).astype(BF)

    def head(u):
        return u // NQ if isinstance(u, int) else lax.shift_right_logical(u, int(math.log2(NQ)))

    def qk(u, s_ref, m_ref):
        h = head(u)
        q2 = qo_v[u]
        m_acc = None
        for j in range(S // CK1):
            s = jnp.dot(k_v[h, j * CK1:(j + 1) * CK1, :], q2, preferred_element_type=F32)
            s_ref[j * CK1:(j + 1) * CK1, :] = s
            mm = jnp.max(s.reshape(CK1 // 8, 8, W), axis=0)
            m_acc = mm if m_acc is None else jnp.maximum(m_acc, mm)
        m_ref[...] = jnp.broadcast_to(jnp.max(m_acc, axis=0, keepdims=True), (8, W))

    def pv(u, s_ref, m_ref):
        h = head(u)
        m = m_ref[0:1, :]
        l_acc = jnp.zeros((8, W), F32)
        acc = jnp.zeros((DH, W), F32)
        for j in range(S // CK2):
            p = jnp.exp2(s_ref[j * CK2:(j + 1) * CK2, :] - m)
            l_acc = l_acc + jnp.sum(p.reshape(CK2 // 8, 8, W), axis=0)
            acc = acc + jnp.dot(vt_v[h, :, j * CK2:(j + 1) * CK2], p.astype(BF), preferred_element_type=F32)
        l = jnp.sum(l_acc, axis=0, keepdims=True)
        qo_v[u] = (acc * (1.0 / l)).astype(BF)

    with jax.named_scope('kfwait'):
        for h in range(4, HKV):
            cp_k(h).start()
        cp_f(6).start()
        for i in range(6):
            cp_f(i).wait()
        cp_k(0).wait()
        cp_v(0).wait()
        cp_v(1).wait()
    with jax.named_scope('qk0_ffn'):
        qk(0, sa_v, ma_v)
        vt_v[0] = v_v[0].T
        vt_v[1] = v_v[1].T
        router_ffn()

    def p2_body(v, c):
        par = lax.bitwise_and(v, 1)

        @pl.when(lax.bitwise_and(v, NQ - 1) == 0)
        def _():
            cp_k(head(v)).wait()

        @pl.when(par == 1)
        def _():
            qk(v, sb_v, mb_v)
            pv(v - 1, sa_v, ma_v)

        @pl.when(par == 0)
        def _():
            qk(v, sa_v, ma_v)
            pv(v - 1, sb_v, mb_v)
        return c
    with jax.named_scope('p2'):
        lax.fori_loop(1, U, p2_body, 0)
    with jax.named_scope('pvlast'):
        scatter_update()
        pv(U - 1, sb_v, mb_v)

    def p3_body(b, c):
        for sub in range(NSUB):
            tok0 = b * TB + sub * SUB
            i = lax.shift_right_logical(tok0, int(math.log2(TQ)))
            t0 = lax.bitwise_and(tok0, TQ - 1)
            parts = []
            for h in range(HKV):
                for a in range(2):
                    parts.append(qo_v[h * NQ + i, :, pl.ds(pl.multiple_of(a * TQ + t0, 128), SUB)])
            rhs = jnp.concatenate(parts, axis=0)
            s_t = jnp.dot(wot_v[...], rhs, preferred_element_type=F32)
            cols = pl.ds(pl.multiple_of(tok0, 128), SUB)
            bo = xnt_v[:, cols].astype(F32)
            g = bo * _sigmoid(bo)
            os_v[b, sub] = (xt_v[:, cols].astype(F32) + s_t * g).astype(BF)
            cp_o(b, sub).start()
        return c
    cp_f(6).wait()
    with jax.named_scope('p3'):
        lax.fori_loop(0, NB, p3_body, 0)
    with jax.named_scope('fin'):
        for bb in range(NB):
            for sub in range(NSUB):
                cp_o(bb, sub).wait()


_SCRATCH = [
    pltpu.VMEM((D, S), BF),
    pltpu.VMEM((D, S), BF),
    pltpu.VMEM((HKV, S, DH), BF),
    pltpu.VMEM((HKV, S, DH), BF),
    pltpu.VMEM((HKV, DH, S), BF),
    pltpu.VMEM((HKV, D, 256), BF),
    pltpu.VMEM((256, D), BF),
    pltpu.VMEM((D, 2 * HKV * DH), BF),
    pltpu.VMEM((U, DH, W), BF),
    pltpu.VMEM((S, W), F32),
    pltpu.VMEM((S, W), F32),
    pltpu.VMEM((8, W), F32),
    pltpu.VMEM((8, W), F32),
    pltpu.VMEM((D, F), BF),
    pltpu.VMEM((D, F), BF),
    pltpu.VMEM((D, F), BF),
    pltpu.VMEM((NB, NSUB, D, SUB), BF),
    pltpu.VMEM((C, S), F32),
    pltpu.VMEM((D, C), F32),
    pltpu.SMEM((C,), jnp.int32),
    pltpu.SemaphoreType.DMA((NLN,)),
    pltpu.SemaphoreType.DMA((HKV,)),
    pltpu.SemaphoreType.DMA((HKV,)),
    pltpu.SemaphoreType.DMA((HKV,)),
    pltpu.SemaphoreType.DMA((7,)),
    pltpu.SemaphoreType.DMA((NB * NSUB,)),
]


def _run(A_x, A_k_cache, A_v_cache, A_wq, A_wo, B_x, B_w_r, B_w_gate, B_w_up, B_w_down):
    any_spec = pl.BlockSpec(memory_space=pl.ANY)
    out_t = pl.pallas_call(
        _kernel,
        in_specs=[any_spec] * 8 + [pl.BlockSpec(memory_space=pltpu.VMEM)],
        out_specs=any_spec,
        out_shape=jax.ShapeDtypeStruct((D, S), BF),
        scratch_shapes=_SCRATCH,
        compiler_params=pltpu.CompilerParams(vmem_limit_bytes=126 * 1024 * 1024,
                                             disable_bounds_checks=True),
    )(A_x.reshape(S, D).T, A_k_cache.reshape(HKV, S, DH), A_v_cache.reshape(HKV, S, DH),
      A_wq, A_wo.T, B_w_gate, B_w_up, B_w_down.T, B_w_r)
    return out_t.T.reshape(1, S, D)


@jax.jit
def pallas_recurrent_scan__gqa_block_cached__moe_arch_mod__prompt_kernel(
    A_x: jax.Array,
    A_k_cache: jax.Array,
    A_v_cache: jax.Array,
    A_wq: jax.Array,
    A_wo: jax.Array,
    B_x: jax.Array,
    B_w_r: jax.Array,
    B_w_gate: jax.Array,
    B_w_up: jax.Array,
    B_w_down: jax.Array,
):
    return _run(A_x, A_k_cache, A_v_cache, A_wq, A_wo, B_x, B_w_r, B_w_gate, B_w_up, B_w_down)
```

```python
import math

import jax
import jax.numpy as jnp
from jax import lax
from jax.experimental import pallas as pl
from jax.experimental.pallas import tpu as pltpu

S = 2048
D = 576
HKV = 16
DH = 128
F = 4608
C = 8
EPS = 1e-5

TQ = 1024
NQ = S // TQ
W = 2 * TQ
U = HKV * NQ
CK1 = 1024
CK2 = 256
LNB = 128
NLN = S // LNB
XW = (0, 2, 4, 8)
TB = 512
SUB = 128
NB = S // TB
NSUB = TB // SUB
NSLAB = 6
FS = F // NSLAB
NT1 = HKV // 2
QSCALE = (DH ** -0.5) * math.log2(math.e)

NT = (((1,), (1,)), ((), ()))
BF = jnp.bfloat16
F32 = jnp.float32


def _rb(x):
    return x.astype(BF).astype(F32)


def _sigmoid(x):
    return 1.0 / (1.0 + jnp.exp(-x))


def _kernel(xt_hbm, k_hbm, v_hbm, wq_hbm, wot_hbm, wg_hbm, wu_hbm, wdt_hbm, wr_ref,
            o_hbm,
            xt_v, xnt_v, k_v, v_v, vt_v, wq_v, wqt_v, wot_v, qo_v,
            sa_v, sb_v, ma_v, mb_v, wg_v, wu_v, wdt_v, wd_v, os_v, r_v, yt_v, idx_s,
            sem_x, sem_wq, sem_v, sem_k, sem_f, sem_d, sem_o):

    def cp_x(b):
        cols = pl.ds(b * LNB, LNB)
        return pltpu.make_async_copy(xt_hbm.at[:, cols], xt_v.at[:, cols], sem_x.at[b])

    def cp_wq(h):
        off = h * 256 if isinstance(h, int) else pl.multiple_of(h * 256, 256)
        return pltpu.make_async_copy(wq_hbm.at[:, pl.ds(off, 256)], wq_v.at[h], sem_wq.at[h])

    def cp_v(h):
        return pltpu.make_async_copy(v_hbm.at[h], v_v.at[h], sem_v.at[h])

    def cp_k(h):
        return pltpu.make_async_copy(k_hbm.at[h], k_v.at[h], sem_k.at[h])

    def cp_f(i):
        if i == 8:
            return pltpu.make_async_copy(wot_hbm, wot_v, sem_f.at[i])
        src, dst = ((wg_hbm, wg_v), (wu_hbm, wu_v))[i // 4]
        cols = pl.ds((i % 4) * (F // 4), F // 4)
        return pltpu.make_async_copy(src.at[:, cols], dst.at[:, cols], sem_f.at[i])

    def cp_d(s):
        off = s * FS if isinstance(s, int) else pl.multiple_of(s * FS, FS)
        cols = pl.ds(off, FS)
        return pltpu.make_async_copy(wdt_hbm.at[:, cols], wdt_v.at[:, cols], sem_d.at[s])

    def cp_o(b, sub):
        off = b * TB + sub * SUB
        off = off if isinstance(off, int) else pl.multiple_of(off, SUB)
        return pltpu.make_async_copy(
            os_v.at[b, sub], o_hbm.at[:, pl.ds(off, SUB)], sem_o.at[b * NSUB + sub])

    def layernorm(b):
        cols = slice(b * LNB, (b + 1) * LNB)
        x = xt_v[:, cols].astype(F32)
        mean = jnp.sum(x, axis=0, keepdims=True) * (1.0 / D)
        xc = x - mean
        var = jnp.sum(xc * xc, axis=0, keepdims=True) * (1.0 / D)
        den = _rb(jnp.sqrt(_rb(_rb(var) + EPS)))
        xn = (_rb(x - _rb(mean)) * (1.0 / den)).astype(BF)
        xnt_v[:, cols] = xn
        return xn

    def store_q(h, qt, c0, n):
        qt = (qt * QSCALE).astype(BF)
        step = min(n, TQ)
        for o in range(0, n, step):
            i, t0 = (c0 + o) // TQ, (c0 + o) % TQ
            for a in range(2):
                qo_v[h * NQ + i, :, a * TQ + t0:a * TQ + t0 + step] = qt[a * DH:(a + 1) * DH, o:o + step]

    with jax.named_scope('p1first'):
        cp_wq(0).start()
        cp_x(0).start()
        cp_wq(1).start()
        cp_x(1).start()
        wr16 = jnp.broadcast_to(wr_ref[...].reshape(1, D), (16, D))
        wdt_v[:, (NSLAB - 1) * FS:] = jnp.zeros((D, FS), BF)
        cp_wq(0).wait()
        wqt_v[...] = wq_v[0].T
        cp_x(0).wait()
        for b in range(2, NLN):
            cp_x(b).start()
        cp_wq(2).start()
        xn = layernorm(0)
        wqt = [wqt_v[...], None]
        store_q(0, jnp.dot(wqt[0], xn, preferred_element_type=F32), 0, LNB)
        for b in range(NLN):
            if b in XW:
                nxt = min([w for w in XW if w > b] + [NLN - 1])
                if b == 0:
                    cp_wq(1).wait()
                for bb in range(b + 1, nxt + 1):
                    if bb == NLN - 1:
                        for h in range(3, 5):
                            cp_wq(h).start()
                        for h in range(4):
                            cp_v(h).start()
                        cp_wq(2).wait()
                    cp_x(bb).wait()
            if b == 0:
                wqt[1] = jnp.concatenate([wq_v[1].T, wr16], axis=0)
            if b + 1 < NLN:
                xn_next = layernorm(b + 1)
            for h in range(2):
                if b == 0 and h == 0:
                    continue
                qt = jnp.dot(wqt[h], xn, preferred_element_type=F32)
                if h == 1:
                    r_v[:, b * LNB:(b + 1) * LNB] = _rb(qt[256:256 + C, :])
                    qt = qt[0:256, :]
                store_q(h, qt, b * LNB, LNB)
            xn = xn_next
        wqt_v[...] = wq_v[2].T
        cp_wq(5).start()
        cp_wq(6).start()
        cp_v(4).start()
        cp_v(5).start()
        cp_d(0).start()

    def p1_body(t, c):
        h0 = 2 * t
        h2 = jnp.minimum(h0 + 2, HKV - 1)

        @pl.when(t < NT1 - 1)
        def _():
            cp_wq(h0 + 2).wait()
        cp_wq(h0 + 1).wait()
        cp_v(h0).wait()
        cp_v(h0 + 1).wait()

        @pl.when(t >= 2)
        def _():
            cp_d(t - 2).wait()
        store_q(h0, jnp.dot(wqt_v[...], xnt_v[...], preferred_element_type=F32), 0, S)
        store_q(h0 + 1, jnp.dot(wq_v[h0 + 1].T, xnt_v[...], preferred_element_type=F32), 0, S)
        wqt_v[...] = wq_v[h2].T
        vt_v[h0] = v_v[h0].T
        vt_v[h0 + 1] = v_v[h0 + 1].T
        d0 = pl.multiple_of(jnp.where(t >= 2, t - 2, NSLAB - 1) * FS, FS)
        wd_v[pl.ds(d0, FS), :] = wdt_v[:, pl.ds(d0, FS)].T

        @pl.when(t < NT1 - 2)
        def _():
            cp_wq(h0 + 5).start()
            cp_v(h0 + 4).start()
            cp_v(h0 + 5).start()

        @pl.when(t < NT1 - 3)
        def _():
            cp_wq(h0 + 6).start()
        @pl.when(t < NSLAB)
        def _():
            cp_d(t).start()
        for i in range(8):
            @pl.when(t == min(1 + i, NT1 - 2))
            def _():
                cp_f(i).start()
        for g in range(2):
            @pl.when(t == NT1 - 3 + g)
            def _():
                cp_k(2 * g).start()
                cp_k(2 * g + 1).start()
        return c
    with jax.named_scope('p1'):
        lax.fori_loop(1, NT1, p1_body, 0)

    def router_ffn():
        r = r_v[...]
        tok = lax.broadcasted_iota(jnp.int32, (C, S), 1).astype(F32)
        row = lax.broadcasted_iota(jnp.int32, (C, 1), 0)
        idx = jnp.zeros((C, 1), F32)
        val = jnp.zeros((C, 1), F32)
        for c in range(C):
            mx = jnp.max(r, axis=1, keepdims=True)
            ix = jnp.min(jnp.where(r == mx, tok, float(S)), axis=1, keepdims=True)
            r = jnp.where(tok == ix, -jnp.inf, r)
            idx = jnp.where(row == c, ix, idx)
            val = jnp.where(row == c, mx, val)
        idx_i = jnp.minimum(idx, float(S - 1)).astype(jnp.int32)
        for c in range(C):
            idx_s[c] = idx_i[c, 0]
        onehot = jnp.where(tok == idx, 1.0, 0.0).astype(BF)
        xs = lax.dot_general(onehot, xnt_v[...], NT, preferred_element_type=F32).astype(BF)
        g = _rb(jnp.dot(xs, wg_v[...], preferred_element_type=F32))
        g = _rb(g * _sigmoid(g))
        u = _rb(jnp.dot(xs, wu_v[...], preferred_element_type=F32))
        hh = (g * u).astype(BF)
        y = _rb(jnp.dot(hh, wd_v[...], preferred_element_type=F32))
        y = _rb(y * _rb(_sigmoid(val)))
        yt_v[...] = y.T

    def scatter_update():
        lane = lax.broadcasted_iota(jnp.int32, (1, 128), 1)
        for c in range(C):
            t = idx_s[c]
            cols = pl.ds(pl.multiple_of(lax.shift_right_logical(t, 7) * 128, 128), 128)
            xb = xnt_v[:, cols].astype(F32)
            hit = lane == lax.bitwise_and(t, 127)
            xnt_v[:, cols] = jnp.where(hit, xb + yt_v[:, c:c + 1], xb).astype(BF)

    def head(u):
        return u // NQ if isinstance(u, int) else lax.shift_right_logical(u, int(math.log2(NQ)))

    def qk(u, s_ref, m_ref):
        h = head(u)
        q2 = qo_v[u]
        m_acc = None
        for j in range(S // CK1):
            s = jnp.dot(k_v[h, j * CK1:(j + 1) * CK1, :], q2, preferred_element_type=F32)
            s_ref[j * CK1:(j + 1) * CK1, :] = s
            mm = jnp.max(s.reshape(CK1 // 8, 8, W), axis=0)
            m_acc = mm if m_acc is None else jnp.maximum(m_acc, mm)
        m_ref[...] = jnp.broadcast_to(jnp.max(m_acc, axis=0, keepdims=True), (8, W))

    def pv(u, s_ref, m_ref):
        h = head(u)
        m = m_ref[0:1, :]
        l_acc = jnp.zeros((8, W), F32)
        acc = jnp.zeros((DH, W), F32)
        for j in range(S // CK2):
            p = jnp.exp2(s_ref[j * CK2:(j + 1) * CK2, :] - m)
            l_acc = l_acc + jnp.sum(p.reshape(CK2 // 8, 8, W), axis=0)
            acc = acc + jnp.dot(vt_v[h, :, j * CK2:(j + 1) * CK2], p.astype(BF), preferred_element_type=F32)
        l = jnp.sum(l_acc, axis=0, keepdims=True)
        qo_v[u] = (acc * (1.0 / l)).astype(BF)

    with jax.named_scope('kfwait'):
        for h in range(4, HKV):
            cp_k(h).start()
        cp_f(8).start()
        for i in range(8):
            cp_f(i).wait()
        cp_k(0).wait()
        cp_v(0).wait()
        cp_v(1).wait()
    with jax.named_scope('qk0_ffn'):
        qk(0, sa_v, ma_v)
        vt_v[0] = v_v[0].T
        vt_v[1] = v_v[1].T
        router_ffn()

    def p2_body(v, c):
        par = lax.bitwise_and(v, 1)

        @pl.when(lax.bitwise_and(v, NQ - 1) == 0)
        def _():
            cp_k(head(v)).wait()

        @pl.when(par == 1)
        def _():
            qk(v, sb_v, mb_v)
            pv(v - 1, sa_v, ma_v)

        @pl.when(par == 0)
        def _():
            qk(v, sa_v, ma_v)
            pv(v - 1, sb_v, mb_v)
        return c
    with jax.named_scope('p2'):
        lax.fori_loop(1, U, p2_body, 0)
    with jax.named_scope('pvlast'):
        scatter_update()
        pv(U - 1, sb_v, mb_v)

    def p3_body(b, c):
        for sub in range(NSUB):
            tok0 = b * TB + sub * SUB
            i = lax.shift_right_logical(tok0, int(math.log2(TQ)))
            t0 = lax.bitwise_and(tok0, TQ - 1)
            parts = []
            for h in range(HKV):
                for a in range(2):
                    parts.append(qo_v[h * NQ + i, :, pl.ds(pl.multiple_of(a * TQ + t0, 128), SUB)])
            rhs = jnp.concatenate(parts, axis=0)
            s_t = jnp.dot(wot_v[...], rhs, preferred_element_type=F32)
            cols = pl.ds(pl.multiple_of(tok0, 128), SUB)
            bo = xnt_v[:, cols].astype(F32)
            g = bo * _sigmoid(bo)
            os_v[b, sub] = (xt_v[:, cols].astype(F32) + s_t * g).astype(BF)
            cp_o(b, sub).start()
        return c
    cp_f(8).wait()
    with jax.named_scope('p3'):
        lax.fori_loop(0, NB, p3_body, 0)
    with jax.named_scope('fin'):
        for bb in range(NB):
            for sub in range(NSUB):
                cp_o(bb, sub).wait()


_SCRATCH = [
    pltpu.VMEM((D, S), BF),
    pltpu.VMEM((D, S), BF),
    pltpu.VMEM((HKV, S, DH), BF),
    pltpu.VMEM((HKV, S, DH), BF),
    pltpu.VMEM((HKV, DH, S), BF),
    pltpu.VMEM((HKV, D, 256), BF),
    pltpu.VMEM((256, D), BF),
    pltpu.VMEM((D, 2 * HKV * DH), BF),
    pltpu.VMEM((U, DH, W), BF),
    pltpu.VMEM((S, W), F32),
    pltpu.VMEM((S, W), F32),
    pltpu.VMEM((8, W), F32),
    pltpu.VMEM((8, W), F32),
    pltpu.VMEM((D, F), BF),
    pltpu.VMEM((D, F), BF),
    pltpu.VMEM((D, F), BF),
    pltpu.VMEM((F, D), BF),
    pltpu.VMEM((NB, NSUB, D, SUB), BF),
    pltpu.VMEM((C, S), F32),
    pltpu.VMEM((D, C), F32),
    pltpu.SMEM((C,), jnp.int32),
    pltpu.SemaphoreType.DMA((NLN,)),
    pltpu.SemaphoreType.DMA((HKV,)),
    pltpu.SemaphoreType.DMA((HKV,)),
    pltpu.SemaphoreType.DMA((HKV,)),
    pltpu.SemaphoreType.DMA((9,)),
    pltpu.SemaphoreType.DMA((NSLAB,)),
    pltpu.SemaphoreType.DMA((NB * NSUB,)),
]


def _run(A_x, A_k_cache, A_v_cache, A_wq, A_wo, B_x, B_w_r, B_w_gate, B_w_up, B_w_down):
    any_spec = pl.BlockSpec(memory_space=pl.ANY)
    out_t = pl.pallas_call(
        _kernel,
        in_specs=[any_spec] * 8 + [pl.BlockSpec(memory_space=pltpu.VMEM)],
        out_specs=any_spec,
        out_shape=jax.ShapeDtypeStruct((D, S), BF),
        scratch_shapes=_SCRATCH,
        compiler_params=pltpu.CompilerParams(vmem_limit_bytes=126 * 1024 * 1024,
                                             disable_bounds_checks=True),
    )(A_x.reshape(S, D).T, A_k_cache.reshape(HKV, S, DH), A_v_cache.reshape(HKV, S, DH),
      A_wq, A_wo.T, B_w_gate, B_w_up, B_w_down.T, B_w_r)
    return out_t.T.reshape(1, S, D)


@jax.jit
def pallas_recurrent_scan__gqa_block_cached__moe_arch_mod__prompt_kernel(
    A_x: jax.Array,
    A_k_cache: jax.Array,
    A_v_cache: jax.Array,
    A_wq: jax.Array,
    A_wo: jax.Array,
    B_x: jax.Array,
    B_w_r: jax.Array,
    B_w_gate: jax.Array,
    B_w_up: jax.Array,
    B_w_down: jax.Array,
):
    return _run(A_x, A_k_cache, A_v_cache, A_wq, A_wo, B_x, B_w_r, B_w_gate, B_w_up, B_w_down)
```

```python
import math

import jax
import jax.numpy as jnp
from jax import lax
from jax.experimental import pallas as pl
from jax.experimental.pallas import tpu as pltpu

S = 2048
D = 576
HKV = 16
DH = 128
F = 4608
C = 8
EPS = 1e-5

TQ = 1024
NQ = S // TQ
W = 2 * TQ
U = HKV * NQ
CK1 = 1024
CK2 = 256
LNB = 128
NLN = S // LNB
XW = (0, 2, 4, 8)
TB = 512
SUB = 128
NB = S // TB
NSUB = TB // SUB
NSLAB = 6
FS = F // NSLAB
NT1 = HKV // 2
QSCALE = (DH ** -0.5) * math.log2(math.e)

NT = (((1,), (1,)), ((), ()))
BF = jnp.bfloat16
F32 = jnp.float32


def _rb(x):
    return x.astype(BF).astype(F32)


def _sigmoid(x):
    return 1.0 / (1.0 + jnp.exp(-x))


def _kernel(xt_hbm, k_hbm, v_hbm, wq_hbm, wot_hbm, wg_hbm, wu_hbm, wdt_hbm, wr_ref,
            o_hbm,
            xt_v, xnt_v, k_v, v_v, vt_v, wq_v, wqt_v, wot_v, qo_v,
            sa_v, sb_v, ma_v, mb_v, wg_v, wu_v, wdt_v, wd_v, os_v, r_v, yt_v, idx_s,
            sem_x, sem_wq, sem_v, sem_k, sem_f, sem_d, sem_o):

    def cp_x(b):
        cols = pl.ds(b * LNB, LNB)
        return pltpu.make_async_copy(xt_hbm.at[:, cols], xt_v.at[:, cols], sem_x.at[b])

    def cp_wq(h):
        off = h * 256 if isinstance(h, int) else pl.multiple_of(h * 256, 256)
        return pltpu.make_async_copy(wq_hbm.at[:, pl.ds(off, 256)], wq_v.at[h], sem_wq.at[h])

    def cp_v(h):
        return pltpu.make_async_copy(v_hbm.at[h], v_v.at[h], sem_v.at[h])

    def cp_k(h):
        return pltpu.make_async_copy(k_hbm.at[h], k_v.at[h], sem_k.at[h])

    def cp_f(i):
        if i == 8:
            return pltpu.make_async_copy(wot_hbm, wot_v, sem_f.at[i])
        src, dst = ((wg_hbm, wg_v), (wu_hbm, wu_v))[i // 4]
        cols = pl.ds((i % 4) * (F // 4), F // 4)
        return pltpu.make_async_copy(src.at[:, cols], dst.at[:, cols], sem_f.at[i])

    def cp_d(s):
        off = s * FS if isinstance(s, int) else pl.multiple_of(s * FS, FS)
        cols = pl.ds(off, FS)
        return pltpu.make_async_copy(wdt_hbm.at[:, cols], wdt_v.at[:, cols], sem_d.at[s])

    def cp_o(b, sub):
        off = b * TB + sub * SUB
        off = off if isinstance(off, int) else pl.multiple_of(off, SUB)
        return pltpu.make_async_copy(
            os_v.at[b, sub], o_hbm.at[:, pl.ds(off, SUB)], sem_o.at[b * NSUB + sub])

    def layernorm(b):
        cols = slice(b * LNB, (b + 1) * LNB)
        x = xt_v[:, cols].astype(F32)
        mean = jnp.sum(x, axis=0, keepdims=True) * (1.0 / D)
        xc = x - mean
        var = jnp.sum(xc * xc, axis=0, keepdims=True) * (1.0 / D)
        den = _rb(jnp.sqrt(_rb(_rb(var) + EPS)))
        xn = (_rb(x - _rb(mean)) * (1.0 / den)).astype(BF)
        xnt_v[:, cols] = xn
        return xn

    def store_q(h, qt, c0, n):
        qt = (qt * QSCALE).astype(BF)
        step = min(n, TQ)
        for o in range(0, n, step):
            i, t0 = (c0 + o) // TQ, (c0 + o) % TQ
            for a in range(2):
                qo_v[h * NQ + i, :, a * TQ + t0:a * TQ + t0 + step] = qt[a * DH:(a + 1) * DH, o:o + step]

    with jax.named_scope('p1first'):
        cp_wq(0).start()
        cp_x(0).start()
        cp_wq(1).start()
        cp_x(1).start()
        wr16 = jnp.broadcast_to(wr_ref[...].reshape(1, D), (16, D))
        wdt_v[:, (NSLAB - 1) * FS:] = jnp.zeros((D, FS), BF)
        cp_wq(0).wait()
        wqt_v[...] = wq_v[0].T
        cp_x(0).wait()
        for b in range(2, NLN):
            cp_x(b).start()
        cp_wq(2).start()
        xn = layernorm(0)
        wqt = [wqt_v[...], None]
        store_q(0, jnp.dot(wqt[0], xn, preferred_element_type=F32), 0, LNB)
        for b in range(NLN):
            if b in XW:
                nxt = min([w for w in XW if w > b] + [NLN - 1])
                if b == 0:
                    cp_wq(1).wait()
                for bb in range(b + 1, nxt + 1):
                    if bb == NLN - 1:
                        for h in range(3, 5):
                            cp_wq(h).start()
                        for h in range(4):
                            cp_v(h).start()
                        cp_wq(2).wait()
                    cp_x(bb).wait()
            if b == 0:
                wqt[1] = jnp.concatenate([wq_v[1].T, wr16], axis=0)
            if b + 1 < NLN:
                xn_next = layernorm(b + 1)
            for h in range(2):
                if b == 0 and h == 0:
                    continue
                qt = jnp.dot(wqt[h], xn, preferred_element_type=F32)
                if h == 1:
                    r_v[:, b * LNB:(b + 1) * LNB] = _rb(qt[256:256 + C, :])
                    qt = qt[0:256, :]
                store_q(h, qt, b * LNB, LNB)
            xn = xn_next
        wqt_v[...] = wq_v[2].T
        cp_wq(5).start()
        cp_wq(6).start()
        cp_v(4).start()
        cp_v(5).start()
        cp_d(0).start()

    def p1_body(t, c):
        h0 = 2 * t
        h2 = jnp.minimum(h0 + 2, HKV - 1)

        @pl.when(t < NT1 - 1)
        def _():
            cp_wq(h0 + 2).wait()
        cp_wq(h0 + 1).wait()
        cp_v(h0).wait()
        cp_v(h0 + 1).wait()

        @pl.when(t >= 2)
        def _():
            cp_d(t - 2).wait()
        store_q(h0, jnp.dot(wqt_v[...], xnt_v[...], preferred_element_type=F32), 0, S)
        store_q(h0 + 1, jnp.dot(wq_v[h0 + 1].T, xnt_v[...], preferred_element_type=F32), 0, S)
        wqt_v[...] = wq_v[h2].T
        vt_v[h0] = v_v[h0].T
        vt_v[h0 + 1] = v_v[h0 + 1].T
        d0 = pl.multiple_of(jnp.where(t >= 2, t - 2, NSLAB - 1) * FS, FS)
        wd_v[pl.ds(d0, FS), :] = wdt_v[:, pl.ds(d0, FS)].T

        @pl.when(t < NT1 - 2)
        def _():
            cp_wq(h0 + 5).start()
            cp_v(h0 + 4).start()
            cp_v(h0 + 5).start()

        @pl.when(t < NT1 - 3)
        def _():
            cp_wq(h0 + 6).start()
        @pl.when(t < NSLAB)
        def _():
            cp_d(t).start()
        for i in range(8):
            @pl.when(t == min(1 + i, NT1 - 2))
            def _():
                cp_f(i).start()
        for g in range(2):
            @pl.when(t == NT1 - 3 + g)
            def _():
                cp_k(2 * g).start()
                cp_k(2 * g + 1).start()
        return c
    with jax.named_scope('p1'):
        lax.fori_loop(1, NT1, p1_body, 0)

    def router_ffn():
        r = r_v[...]
        tok = lax.broadcasted_iota(jnp.int32, (C, S), 1).astype(F32)
        row = lax.broadcasted_iota(jnp.int32, (C, 1), 0)
        idx = jnp.zeros((C, 1), F32)
        val = jnp.zeros((C, 1), F32)
        for c in range(C):
            mx = jnp.max(r, axis=1, keepdims=True)
            ix = jnp.min(jnp.where(r == mx, tok, float(S)), axis=1, keepdims=True)
            r = jnp.where(tok == ix, -jnp.inf, r)
            idx = jnp.where(row == c, ix, idx)
            val = jnp.where(row == c, mx, val)
        idx_i = jnp.minimum(idx, float(S - 1)).astype(jnp.int32)
        for c in range(C):
            idx_s[c] = idx_i[c, 0]
        onehot = jnp.where(tok == idx, 1.0, 0.0).astype(BF)
        xs = lax.dot_general(onehot, xnt_v[...], NT, preferred_element_type=F32).astype(BF)
        g = _rb(jnp.dot(xs, wg_v[...], preferred_element_type=F32))
        g = _rb(g * _sigmoid(g))
        u = _rb(jnp.dot(xs, wu_v[...], preferred_element_type=F32))
        hh = (g * u).astype(BF)
        y = _rb(jnp.dot(hh, wd_v[...], preferred_element_type=F32))
        y = _rb(y * _rb(_sigmoid(val)))
        yt_v[...] = y.T

    def scatter_update():
        lane = lax.broadcasted_iota(jnp.int32, (1, 128), 1)
        for c in range(C):
            t = idx_s[c]
            cols = pl.ds(pl.multiple_of(lax.shift_right_logical(t, 7) * 128, 128), 128)
            xb = xnt_v[:, cols].astype(F32)
            hit = lane == lax.bitwise_and(t, 127)
            xnt_v[:, cols] = jnp.where(hit, xb + yt_v[:, c:c + 1], xb).astype(BF)

    def head(u):
        return u // NQ if isinstance(u, int) else lax.shift_right_logical(u, int(math.log2(NQ)))

    def qk(u, s_ref, m_ref):
        h = head(u)
        q2 = qo_v[u]
        m_acc = None
        for j in range(S // CK1):
            s = jnp.dot(k_v[h, j * CK1:(j + 1) * CK1, :], q2, preferred_element_type=F32)
            s_ref[j * CK1:(j + 1) * CK1, :] = s
            mm = jnp.max(s.reshape(CK1 // 8, 8, W), axis=0)
            m_acc = mm if m_acc is None else jnp.maximum(m_acc, mm)
        m_ref[...] = jnp.broadcast_to(jnp.max(m_acc, axis=0, keepdims=True), (8, W))

    def pv(u, s_ref, m_ref):
        h = head(u)
        m = m_ref[0:1, :]
        l_acc = jnp.zeros((8, W), F32)
        acc = jnp.zeros((DH, W), F32)
        for j in range(S // CK2):
            p = jnp.exp2(s_ref[j * CK2:(j + 1) * CK2, :] - m)
            l_acc = l_acc + jnp.sum(p.reshape(CK2 // 8, 8, W), axis=0)
            acc = acc + jnp.dot(vt_v[h, :, j * CK2:(j + 1) * CK2], p.astype(BF), preferred_element_type=F32)
        l = jnp.sum(l_acc, axis=0, keepdims=True)
        qo_v[u] = (acc * (1.0 / l)).astype(BF)

    with jax.named_scope('kfwait'):
        for h in range(4, HKV):
            cp_k(h).start()
        cp_f(8).start()
        for i in range(8):
            cp_f(i).wait()
        cp_k(0).wait()
        cp_v(0).wait()
        cp_v(1).wait()
    with jax.named_scope('qk0_ffn'):
        qk(0, sa_v, ma_v)
        vt_v[0] = v_v[0].T
        vt_v[1] = v_v[1].T
        router_ffn()

    def p2_body(v, c):
        par = lax.bitwise_and(v, 1)

        @pl.when(lax.bitwise_and(v, NQ - 1) == 0)
        def _():
            cp_k(head(v)).wait()

        @pl.when(par == 1)
        def _():
            qk(v, sb_v, mb_v)
            pv(v - 1, sa_v, ma_v)

        @pl.when(par == 0)
        def _():
            qk(v, sa_v, ma_v)
            pv(v - 1, sb_v, mb_v)
        return c
    with jax.named_scope('p2'):
        lax.fori_loop(1, U, p2_body, 0)
    def p3_block(b):
        for sub in range(NSUB):
            tok0 = b * TB + sub * SUB
            if isinstance(b, int):
                i, t0 = tok0 // TQ, tok0 % TQ
                al = lambda x: x
            else:
                i = lax.shift_right_logical(tok0, int(math.log2(TQ)))
                t0 = lax.bitwise_and(tok0, TQ - 1)
                al = lambda x: pl.multiple_of(x, 128)
            parts = []
            for h in range(HKV):
                for a in range(2):
                    parts.append(qo_v[h * NQ + i, :, pl.ds(al(a * TQ + t0), SUB)])
            rhs = jnp.concatenate(parts, axis=0)
            s_t = jnp.dot(wot_v[...], rhs, preferred_element_type=F32)
            cols = pl.ds(al(tok0), SUB)
            bo = xnt_v[:, cols].astype(F32)
            g = bo * _sigmoid(bo)
            os_v[b, sub] = (xt_v[:, cols].astype(F32) + s_t * g).astype(BF)
            cp_o(b, sub).start()

    def p3_body(b, c):
        p3_block(b)
        return c
    cp_f(8).wait()
    with jax.named_scope('pvlast'):
        scatter_update()
        pv(U - 1, sb_v, mb_v)
        p3_block(0)
    with jax.named_scope('p3'):
        lax.fori_loop(1, NB, p3_body, 0)
    with jax.named_scope('fin'):
        for bb in range(NB):
            for sub in range(NSUB):
                cp_o(bb, sub).wait()


_SCRATCH = [
    pltpu.VMEM((D, S), BF),
    pltpu.VMEM((D, S), BF),
    pltpu.VMEM((HKV, S, DH), BF),
    pltpu.VMEM((HKV, S, DH), BF),
    pltpu.VMEM((HKV, DH, S), BF),
    pltpu.VMEM((HKV, D, 256), BF),
    pltpu.VMEM((256, D), BF),
    pltpu.VMEM((D, 2 * HKV * DH), BF),
    pltpu.VMEM((U, DH, W), BF),
    pltpu.VMEM((S, W), F32),
    pltpu.VMEM((S, W), F32),
    pltpu.VMEM((8, W), F32),
    pltpu.VMEM((8, W), F32),
    pltpu.VMEM((D, F), BF),
    pltpu.VMEM((D, F), BF),
    pltpu.VMEM((D, F), BF),
    pltpu.VMEM((F, D), BF),
    pltpu.VMEM((NB, NSUB, D, SUB), BF),
    pltpu.VMEM((C, S), F32),
    pltpu.VMEM((D, C), F32),
    pltpu.SMEM((C,), jnp.int32),
    pltpu.SemaphoreType.DMA((NLN,)),
    pltpu.SemaphoreType.DMA((HKV,)),
    pltpu.SemaphoreType.DMA((HKV,)),
    pltpu.SemaphoreType.DMA((HKV,)),
    pltpu.SemaphoreType.DMA((9,)),
    pltpu.SemaphoreType.DMA((NSLAB,)),
    pltpu.SemaphoreType.DMA((NB * NSUB,)),
]


def _run(A_x, A_k_cache, A_v_cache, A_wq, A_wo, B_x, B_w_r, B_w_gate, B_w_up, B_w_down):
    any_spec = pl.BlockSpec(memory_space=pl.ANY)
    out_t = pl.pallas_call(
        _kernel,
        in_specs=[any_spec] * 8 + [pl.BlockSpec(memory_space=pltpu.VMEM)],
        out_specs=any_spec,
        out_shape=jax.ShapeDtypeStruct((D, S), BF),
        scratch_shapes=_SCRATCH,
        compiler_params=pltpu.CompilerParams(vmem_limit_bytes=126 * 1024 * 1024,
                                             disable_bounds_checks=True),
    )(A_x.reshape(S, D).T, A_k_cache.reshape(HKV, S, DH), A_v_cache.reshape(HKV, S, DH),
      A_wq, A_wo.T, B_w_gate, B_w_up, B_w_down.T, B_w_r)
    return out_t.T.reshape(1, S, D)


@jax.jit
def pallas_recurrent_scan__gqa_block_cached__moe_arch_mod__prompt_kernel(
    A_x: jax.Array,
    A_k_cache: jax.Array,
    A_v_cache: jax.Array,
    A_wq: jax.Array,
    A_wo: jax.Array,
    B_x: jax.Array,
    B_w_r: jax.Array,
    B_w_gate: jax.Array,
    B_w_up: jax.Array,
    B_w_down: jax.Array,
):
    return _run(A_x, A_k_cache, A_v_cache, A_wq, A_wo, B_x, B_w_r, B_w_gate, B_w_up, B_w_down)
```

```python
import math

import jax
import jax.numpy as jnp
from jax import lax
from jax.experimental import pallas as pl
from jax.experimental.pallas import tpu as pltpu

S = 2048
D = 576
HKV = 16
DH = 128
F = 4608
C = 8
EPS = 1e-5

TQ = 1024
NQ = S // TQ
W = 2 * TQ
U = HKV * NQ
CK1 = 1024
CK2 = 256
LNB = 128
NLN = S // LNB
XW = (0, 2, 4, 8)
TB = 512
SUB = 128
NB = S // TB
NSUB = TB // SUB
NSLAB = 6
FS = F // NSLAB
NT1 = HKV // 2
QSCALE = (DH ** -0.5) * math.log2(math.e)

NT = (((1,), (1,)), ((), ()))
BF = jnp.bfloat16
F32 = jnp.float32


def _rb(x):
    return x.astype(BF).astype(F32)


def _sigmoid(x):
    return 1.0 / (1.0 + jnp.exp(-x))


def _kernel(xt_hbm, k_hbm, v_hbm, wq_hbm, wot_hbm, wg_hbm, wu_hbm, wdt_hbm, wr_hbm,
            o_hbm,
            xt_v, xnt_v, k_v, v_v, vt_v, wq_v, wqt_v, wot_v, qo_v,
            sa_v, sb_v, ma_v, mb_v, wg_v, wu_v, wdt_v, wd_v, os_v, wr_v, r_v, yt_v, idx_s,
            sem_x, sem_wq, sem_v, sem_k, sem_f, sem_d, sem_r, sem_o):

    def cp_x(b):
        cols = pl.ds(b * LNB, LNB)
        return pltpu.make_async_copy(xt_hbm.at[:, cols], xt_v.at[:, cols], sem_x.at[b])

    def cp_wq(h):
        off = h * 256 if isinstance(h, int) else pl.multiple_of(h * 256, 256)
        return pltpu.make_async_copy(wq_hbm.at[:, pl.ds(off, 256)], wq_v.at[h], sem_wq.at[h])

    def cp_v(h):
        return pltpu.make_async_copy(v_hbm.at[h], v_v.at[h], sem_v.at[h])

    def cp_k(h):
        return pltpu.make_async_copy(k_hbm.at[h], k_v.at[h], sem_k.at[h])

    def cp_f(i):
        if i == 8:
            return pltpu.make_async_copy(wot_hbm, wot_v, sem_f.at[i])
        src, dst = ((wg_hbm, wg_v), (wu_hbm, wu_v))[i // 4]
        cols = pl.ds((i % 4) * (F // 4), F // 4)
        return pltpu.make_async_copy(src.at[:, cols], dst.at[:, cols], sem_f.at[i])

    def cp_d(s):
        off = s * FS if isinstance(s, int) else pl.multiple_of(s * FS, FS)
        cols = pl.ds(off, FS)
        return pltpu.make_async_copy(wdt_hbm.at[:, cols], wdt_v.at[:, cols], sem_d.at[s])

    def cp_r():
        return pltpu.make_async_copy(wr_hbm, wr_v, sem_r.at[0])

    def cp_o(b, sub):
        off = b * TB + sub * SUB
        off = off if isinstance(off, int) else pl.multiple_of(off, SUB)
        return pltpu.make_async_copy(
            os_v.at[b, sub], o_hbm.at[:, pl.ds(off, SUB)], sem_o.at[b * NSUB + sub])

    def layernorm(b):
        cols = slice(b * LNB, (b + 1) * LNB)
        x = xt_v[:, cols].astype(F32)
        mean = jnp.sum(x, axis=0, keepdims=True) * (1.0 / D)
        xc = x - mean
        var = jnp.sum(xc * xc, axis=0, keepdims=True) * (1.0 / D)
        den = _rb(jnp.sqrt(_rb(_rb(var) + EPS)))
        xn = (_rb(x - _rb(mean)) * (1.0 / den)).astype(BF)
        xnt_v[:, cols] = xn
        return xn

    def store_q(h, qt, c0, n):
        qt = (qt * QSCALE).astype(BF)
        step = min(n, TQ)
        for o in range(0, n, step):
            i, t0 = (c0 + o) // TQ, (c0 + o) % TQ
            for a in range(2):
                qo_v[h * NQ + i, :, a * TQ + t0:a * TQ + t0 + step] = qt[a * DH:(a + 1) * DH, o:o + step]

    with jax.named_scope('p1first'):
        cp_wq(0).start()
        cp_x(0).start()
        cp_wq(1).start()
        cp_x(1).start()
        cp_r().start()
        wdt_v[:, (NSLAB - 1) * FS:] = jnp.zeros((D, FS), BF)
        cp_wq(0).wait()
        wqt_v[...] = wq_v[0].T
        cp_x(0).wait()
        for b in range(2, NLN):
            cp_x(b).start()
        cp_wq(2).start()
        xn = layernorm(0)
        wqt = [wqt_v[...], None]
        store_q(0, jnp.dot(wqt[0], xn, preferred_element_type=F32), 0, LNB)
        for b in range(NLN):
            if b in XW:
                nxt = min([w for w in XW if w > b] + [NLN - 1])
                if b == 0:
                    cp_wq(1).wait()
                    cp_r().wait()
                for bb in range(b + 1, nxt + 1):
                    if bb == NLN - 1:
                        for h in range(3, 5):
                            cp_wq(h).start()
                        for h in range(4):
                            cp_v(h).start()
                        cp_wq(2).wait()
                    cp_x(bb).wait()
            if b == 0:
                wr16 = jnp.broadcast_to(wr_v[...].reshape(1, D), (16, D))
                wqt[1] = jnp.concatenate([wq_v[1].T, wr16], axis=0)
            if b + 1 < NLN:
                xn_next = layernorm(b + 1)
            for h in range(2):
                if b == 0 and h == 0:
                    continue
                qt = jnp.dot(wqt[h], xn, preferred_element_type=F32)
                if h == 1:
                    r_v[:, b * LNB:(b + 1) * LNB] = _rb(qt[256:256 + C, :])
                    qt = qt[0:256, :]
                store_q(h, qt, b * LNB, LNB)
            xn = xn_next
        wqt_v[...] = wq_v[2].T
        cp_wq(5).start()
        cp_wq(6).start()
        cp_v(4).start()
        cp_v(5).start()
        cp_d(0).start()

    def p1_body(t, c):
        h0 = 2 * t
        h2 = jnp.minimum(h0 + 2, HKV - 1)

        @pl.when(t < NT1 - 1)
        def _():
            cp_wq(h0 + 2).wait()
        cp_wq(h0 + 1).wait()
        cp_v(h0).wait()
        cp_v(h0 + 1).wait()

        @pl.when(t >= 2)
        def _():
            cp_d(t - 2).wait()
        store_q(h0, jnp.dot(wqt_v[...], xnt_v[...], preferred_element_type=F32), 0, S)
        store_q(h0 + 1, jnp.dot(wq_v[h0 + 1].T, xnt_v[...], preferred_element_type=F32), 0, S)
        wqt_v[...] = wq_v[h2].T
        vt_v[h0] = v_v[h0].T
        vt_v[h0 + 1] = v_v[h0 + 1].T
        d0 = pl.multiple_of(jnp.where(t >= 2, t - 2, NSLAB - 1) * FS, FS)
        wd_v[pl.ds(d0, FS), :] = wdt_v[:, pl.ds(d0, FS)].T

        @pl.when(t < NT1 - 2)
        def _():
            cp_wq(h0 + 5).start()
            cp_v(h0 + 4).start()
            cp_v(h0 + 5).start()

        @pl.when(t < NT1 - 3)
        def _():
            cp_wq(h0 + 6).start()
        @pl.when(t < NSLAB)
        def _():
            cp_d(t).start()
        for i in range(8):
            @pl.when(t == min(1 + i, NT1 - 2))
            def _():
                cp_f(i).start()
        for g in range(2):
            @pl.when(t == NT1 - 3 + g)
            def _():
                cp_k(2 * g).start()
                cp_k(2 * g + 1).start()
        return c
    with jax.named_scope('p1'):
        lax.fori_loop(1, NT1, p1_body, 0)

    def router_ffn():
        r = r_v[...]
        tok = lax.broadcasted_iota(jnp.int32, (C, S), 1).astype(F32)
        row = lax.broadcasted_iota(jnp.int32, (C, 1), 0)
        idx = jnp.zeros((C, 1), F32)
        val = jnp.zeros((C, 1), F32)
        for c in range(C):
            mx = jnp.max(r, axis=1, keepdims=True)
            ix = jnp.min(jnp.where(r == mx, tok, float(S)), axis=1, keepdims=True)
            r = jnp.where(tok == ix, -jnp.inf, r)
            idx = jnp.where(row == c, ix, idx)
            val = jnp.where(row == c, mx, val)
        idx_i = jnp.minimum(idx, float(S - 1)).astype(jnp.int32)
        for c in range(C):
            idx_s[c] = idx_i[c, 0]
        onehot = jnp.where(tok == idx, 1.0, 0.0).astype(BF)
        xs = lax.dot_general(onehot, xnt_v[...], NT, preferred_element_type=F32).astype(BF)
        g = _rb(jnp.dot(xs, wg_v[...], preferred_element_type=F32))
        g = _rb(g * _sigmoid(g))
        u = _rb(jnp.dot(xs, wu_v[...], preferred_element_type=F32))
        hh = (g * u).astype(BF)
        y = _rb(jnp.dot(hh, wd_v[...], preferred_element_type=F32))
        y = _rb(y * _rb(_sigmoid(val)))
        yt_v[...] = y.T

    def scatter_update():
        lane = lax.broadcasted_iota(jnp.int32, (1, 128), 1)
        for c in range(C):
            t = idx_s[c]
            cols = pl.ds(pl.multiple_of(lax.shift_right_logical(t, 7) * 128, 128), 128)
            xb = xnt_v[:, cols].astype(F32)
            hit = lane == lax.bitwise_and(t, 127)
            xnt_v[:, cols] = jnp.where(hit, xb + yt_v[:, c:c + 1], xb).astype(BF)

    def head(u):
        return u // NQ if isinstance(u, int) else lax.shift_right_logical(u, int(math.log2(NQ)))

    def qk(u, s_ref, m_ref):
        h = head(u)
        q2 = qo_v[u]
        m_acc = None
        for j in range(S // CK1):
            s = jnp.dot(k_v[h, j * CK1:(j + 1) * CK1, :], q2, preferred_element_type=F32)
            s_ref[j * CK1:(j + 1) * CK1, :] = s
            mm = jnp.max(s.reshape(CK1 // 8, 8, W), axis=0)
            m_acc = mm if m_acc is None else jnp.maximum(m_acc, mm)
        m_ref[...] = jnp.broadcast_to(jnp.max(m_acc, axis=0, keepdims=True), (8, W))

    def pv(u, s_ref, m_ref):
        h = head(u)
        m = m_ref[0:1, :]
        l_acc = jnp.zeros((8, W), F32)
        acc = jnp.zeros((DH, W), F32)
        for j in range(S // CK2):
            p = jnp.exp2(s_ref[j * CK2:(j + 1) * CK2, :] - m)
            l_acc = l_acc + jnp.sum(p.reshape(CK2 // 8, 8, W), axis=0)
            acc = acc + jnp.dot(vt_v[h, :, j * CK2:(j + 1) * CK2], p.astype(BF), preferred_element_type=F32)
        l = jnp.sum(l_acc, axis=0, keepdims=True)
        qo_v[u] = (acc * (1.0 / l)).astype(BF)

    with jax.named_scope('kfwait'):
        for h in range(4, HKV):
            cp_k(h).start()
        cp_f(8).start()
        for i in range(8):
            cp_f(i).wait()
        cp_k(0).wait()
        cp_v(0).wait()
        cp_v(1).wait()
    with jax.named_scope('qk0_ffn'):
        qk(0, sa_v, ma_v)
        vt_v[0] = v_v[0].T
        vt_v[1] = v_v[1].T
        router_ffn()

    def p2_body(v, c):
        par = lax.bitwise_and(v, 1)

        @pl.when(lax.bitwise_and(v, NQ - 1) == 0)
        def _():
            cp_k(head(v)).wait()

        @pl.when(par == 1)
        def _():
            qk(v, sb_v, mb_v)
            pv(v - 1, sa_v, ma_v)

        @pl.when(par == 0)
        def _():
            qk(v, sa_v, ma_v)
            pv(v - 1, sb_v, mb_v)
        return c
    with jax.named_scope('p2'):
        lax.fori_loop(1, U, p2_body, 0)
    def p3_block(b):
        for sub in range(NSUB):
            tok0 = b * TB + sub * SUB
            if isinstance(b, int):
                i, t0 = tok0 // TQ, tok0 % TQ
                al = lambda x: x
            else:
                i = lax.shift_right_logical(tok0, int(math.log2(TQ)))
                t0 = lax.bitwise_and(tok0, TQ - 1)
                al = lambda x: pl.multiple_of(x, 128)
            parts = []
            for h in range(HKV):
                for a in range(2):
                    parts.append(qo_v[h * NQ + i, :, pl.ds(al(a * TQ + t0), SUB)])
            rhs = jnp.concatenate(parts, axis=0)
            s_t = jnp.dot(wot_v[...], rhs, preferred_element_type=F32)
            cols = pl.ds(al(tok0), SUB)
            bo = xnt_v[:, cols].astype(F32)
            g = bo * _sigmoid(bo)
            os_v[b, sub] = (xt_v[:, cols].astype(F32) + s_t * g).astype(BF)
            cp_o(b, sub).start()

    def p3_body(b, c):
        p3_block(b)
        return c
    cp_f(8).wait()
    with jax.named_scope('pvlast'):
        scatter_update()
        pv(U - 1, sb_v, mb_v)
        p3_block(0)
    with jax.named_scope('p3'):
        lax.fori_loop(1, NB, p3_body, 0)
    with jax.named_scope('fin'):
        for bb in range(NB):
            for sub in range(NSUB):
                cp_o(bb, sub).wait()


_SCRATCH = [
    pltpu.VMEM((D, S), BF),
    pltpu.VMEM((D, S), BF),
    pltpu.VMEM((HKV, S, DH), BF),
    pltpu.VMEM((HKV, S, DH), BF),
    pltpu.VMEM((HKV, DH, S), BF),
    pltpu.VMEM((HKV, D, 256), BF),
    pltpu.VMEM((256, D), BF),
    pltpu.VMEM((D, 2 * HKV * DH), BF),
    pltpu.VMEM((U, DH, W), BF),
    pltpu.VMEM((S, W), F32),
    pltpu.VMEM((S, W), F32),
    pltpu.VMEM((8, W), F32),
    pltpu.VMEM((8, W), F32),
    pltpu.VMEM((D, F), BF),
    pltpu.VMEM((D, F), BF),
    pltpu.VMEM((D, F), BF),
    pltpu.VMEM((F, D), BF),
    pltpu.VMEM((NB, NSUB, D, SUB), BF),
    pltpu.VMEM((D,), BF),
    pltpu.VMEM((C, S), F32),
    pltpu.VMEM((D, C), F32),
    pltpu.SMEM((C,), jnp.int32),
    pltpu.SemaphoreType.DMA((NLN,)),
    pltpu.SemaphoreType.DMA((HKV,)),
    pltpu.SemaphoreType.DMA((HKV,)),
    pltpu.SemaphoreType.DMA((HKV,)),
    pltpu.SemaphoreType.DMA((9,)),
    pltpu.SemaphoreType.DMA((NSLAB,)),
    pltpu.SemaphoreType.DMA((1,)),
    pltpu.SemaphoreType.DMA((NB * NSUB,)),
]


def _run(A_x, A_k_cache, A_v_cache, A_wq, A_wo, B_x, B_w_r, B_w_gate, B_w_up, B_w_down):
    any_spec = pl.BlockSpec(memory_space=pl.ANY)
    out_t = pl.pallas_call(
        _kernel,
        in_specs=[any_spec] * 9,
        out_specs=any_spec,
        out_shape=jax.ShapeDtypeStruct((D, S), BF),
        scratch_shapes=_SCRATCH,
        compiler_params=pltpu.CompilerParams(vmem_limit_bytes=126 * 1024 * 1024,
                                             disable_bounds_checks=True),
    )(A_x.reshape(S, D).T, A_k_cache.reshape(HKV, S, DH), A_v_cache.reshape(HKV, S, DH),
      A_wq, A_wo.T, B_w_gate, B_w_up, B_w_down.T, B_w_r)
    return out_t.T.reshape(1, S, D)


@jax.jit
def pallas_recurrent_scan__gqa_block_cached__moe_arch_mod__prompt_kernel(
    A_x: jax.Array,
    A_k_cache: jax.Array,
    A_v_cache: jax.Array,
    A_wq: jax.Array,
    A_wo: jax.Array,
    B_x: jax.Array,
    B_w_r: jax.Array,
    B_w_gate: jax.Array,
    B_w_up: jax.Array,
    B_w_down: jax.Array,
):
    return _run(A_x, A_k_cache, A_v_cache, A_wq, A_wo, B_x, B_w_r, B_w_gate, B_w_up, B_w_down)
```
